```python
import jax
import jax.numpy as jnp

def _softmax(x, axis=-1):
    return jax.nn.softmax(x, axis=axis)
def _gelu(x):
    return jax.nn.gelu(x, approximate=True)
def _silu(x):
    return jax.nn.silu(x)
def _sigmoid(x):
    return jax.nn.sigmoid(x)
def _layernorm(x, axis=-1, eps=1e-5):
    m = jnp.mean(x, axis=axis, keepdims=True)
    v = jnp.var(x, axis=axis, keepdims=True)
    return (x - m) / jnp.sqrt(v + eps)
def _scatter_add(tgt, idx, src, axis=0):
    return tgt.at[idx].add(src)
def _segment_sum(src, seg, n):
    return jax.ops.segment_sum(src, seg, n)
class _Rng:
    def __init__(self, key):
        self._k = key
    def _next(self):
        self._k, sub = jax.random.split(self._k)
        return sub
    def normal(self, shape):
        return jax.random.normal(self._next(), shape, dtype=jnp.bfloat16)
    def randint(self, lo, hi, shape):
        return jax.random.randint(self._next(), shape, lo, hi, dtype=jnp.int32)
    def uniform(self, shape, lo=0.0, hi=1.0):
        return jax.random.uniform(self._next(), shape, jnp.bfloat16, lo, hi)
    def permutation(self, n):
        return jax.random.permutation(self._next(), n)


kernel_name = 'interleave_layers__sliding_local_dilated__glu_gated_swiglu__prompt'

def setup_inputs():
    _rng = _Rng(jax.random.key(int.from_bytes(__import__("os").urandom(4), "little")))
    _w = (lambda a: (lambda t: t.astype(jnp.bfloat16) if jnp.issubdtype(t.dtype, jnp.floating) else t)(jnp.asarray(a)))
    def _A_setup():
        B, S, D = 1, 2048, 1024
        return {
            "x": _w((lambda *s: _rng.normal(s) * 0.05)(B, S, D)),
            "wqkv": _w((lambda *s: _rng.normal(s) * 0.05)(D, 3 * D)),
            "wo": _w((lambda *s: _rng.normal(s) * 0.05)(D, D)),
        }
    _A_in = _A_setup()

    def _B_setup():
        B, S, D, F = 1, 2048, 1024, 3584
        return {
            "x": _w((lambda *s: _rng.normal(s) * 0.05)(B, S, D)),
            "w1": _w((lambda *s: _rng.normal(s) * 0.05)(D, F) * (2.0 / D) ** 0.5),
            "w3": _w((lambda *s: _rng.normal(s) * 0.05)(D, F) * (2.0 / D) ** 0.5),
            "w2": _w((lambda *s: _rng.normal(s) * 0.05)(F, D) * (2.0 / F) ** 0.5),
        }
    _B_in = _B_setup()

    return {
        "A_x": _A_in["x"],
        "A_wqkv": _A_in["wqkv"],
        "A_wo": _A_in["wo"],
        "B_x": _B_in["x"],
        "B_w1": _B_in["w1"],
        "B_w3": _B_in["w3"],
        "B_w2": _B_in["w2"],
    }

def reference(A_x, A_wqkv, A_wo, B_x, B_w1, B_w3, B_w2):
    def _A_ref(x, wqkv, wo):
        B, S, D = x.shape
        H = 32; Dh = D // H
        W, dil = 8, 2
        qkv = (lambda x, *d: x.transpose(*d))((x @ wqkv).reshape(B, S, 3, H, Dh), 2, 0, 3, 1, 4)
        q, k, v = qkv[0], qkv[1], qkv[2]
        scale = Dh ** -0.5
        pos = jnp.arange(S)
        off = jnp.arange(W) * dil
        idx = pos[:, None] - off[None, :]
        mask = idx >= 0
        idx_c = jnp.where(mask, idx, 0).reshape(-1)
        kg = k[:, :, idx_c, :].reshape(B, H, S, W, Dh)
        vg = v[:, :, idx_c, :].reshape(B, H, S, W, Dh)
        logits = jnp.einsum("bhsd,bhswd->bhsw", q, kg) * scale
        logits = jnp.where(mask[None, None, :, :], logits, -1e9)
        attn = _softmax(logits, axis=-1)
        o = jnp.einsum("bhsw,bhswd->bhsd", attn, vg)
        return (lambda x, *d: x.transpose(*d))(o, 0, 2, 1, 3).reshape(B, S, D) @ wo

    def _B_ref(x, w1, w3, w2):
        gate = jnp.einsum("bsd,df->bsf", x, w1)
        up = jnp.einsum("bsd,df->bsf", x, w3)
        h = _silu(gate) * up
        out = jnp.einsum("bsf,fd->bsd", h, w2)
        return out

    x = A_x
    x = x + _A_ref(_layernorm(x, axis=-1), A_wqkv, A_wo)
    x = x + _B_ref(_layernorm(x, axis=-1), B_w1, B_w3, B_w2)
    x = x + _A_ref(_layernorm(x, axis=-1), A_wqkv, A_wo)
    x = x + _B_ref(_layernorm(x, axis=-1), B_w1, B_w3, B_w2)
    return x
```

```python
import functools
import jax
import jax.numpy as jnp
import numpy as np
import jax.experimental.pallas as pl
import jax.experimental.pallas.tpu as pltpu

S, D, F = 2048, 1024, 3584
H, DH, W, DIL = 32, 32, 8, 2
HALO = 16
NB = D // 128
f32, bf16 = jnp.float32, jnp.bfloat16


def _ln(x):
    m = jnp.mean(x, axis=-1, keepdims=True)
    d = x - m
    v = jnp.mean(d * d, axis=-1, keepdims=True)
    return d * jax.lax.rsqrt(v + 1e-5)


def _dot(a, b):
    return jnp.dot(a, b, preferred_element_type=f32)


def _swap_blocks(blocks, lane):
    blocks = list(blocks)
    for b in range(3):
        dist = 2 << b
        low = (lane & dist) == 0
        for c in range(NB):
            if c & (1 << b):
                continue
            A, B = blocks[c], blocks[c | (1 << b)]
            blocks[c] = jnp.where(low, A, pltpu.roll(B, dist, 1))
            blocks[c | (1 << b)] = jnp.where(low, pltpu.roll(A, 128 - dist, 1), B)
    return blocks


def make(TM=512, FC=512, R=16, ffn_loop=True, layer_loop=True):
    def kernel(x_ref, wqkv_hbm, wo_hbm, w1_hbm, w3_hbm, w2_hbm, o_ref,
               wqkv, wo_raw, wo, w1, w3, w2, xs, qs, ks, vs, kh, vh, os_, sems):
        step = pl.program_id(0)

        @pl.when(step == 0)
        def _prologue():
            cps = [pltpu.make_async_copy(wqkv_hbm.at[:, pl.ds(i * D, D)], wqkv.at[:, pl.ds(i * D, D)], sems.at[i]) for i in range(3)]
            wo_cps = [pltpu.make_async_copy(wo_hbm.at[:, pl.ds(n * 128, 128)], wo_raw.at[n], sems.at[3]) for n in range(NB)]
            cps.extend(wo_cps)
            cps.append(pltpu.make_async_copy(w1_hbm, w1, sems.at[4]))
            cps.append(pltpu.make_async_copy(w3_hbm, w3, sems.at[5]))
            cps.append(pltpu.make_async_copy(w2_hbm, w2, sems.at[6]))
            for c in cps:
                c.start()
            w32 = wqkv.bitcast(jnp.uint32)
            PR = 32
            lane = jax.lax.broadcasted_iota(jnp.int32, (PR, 128), 1)
            for i in range(3):
                cps[i].wait()

                def body(r, _, i=i):
                    r0 = pl.multiple_of(r * PR, PR)
                    blocks = [w32[pl.ds(r0, PR), pl.ds(i * D + c * 128, 128)] for c in range(NB)]
                    blocks = _swap_blocks(blocks, lane)
                    for c in range(NB):
                        w32[pl.ds(r0, PR), pl.ds(i * D + c * 128, 128)] = blocks[c]
                    return 0
                jax.lax.fori_loop(0, D // 2 // PR, body, 0)
            for c in wo_cps:
                c.wait()
            src = wo_raw.bitcast(jnp.uint32)
            dst = wo.bitcast(jnp.uint32)
            for n in range(NB):
                for j in range(NB):
                    for m in range(8):
                        dst[pl.ds(j * 64 + m * 8, 8), pl.ds(n * 128, 128)] = src[n, pl.ds(m * 8 + j, 8, stride=64), :]
            cps[-3].wait()
            cps[-2].wait()
            cps[-1].wait()
            kh[...] = jnp.zeros(kh.shape, f32)

        xs[...] = x_ref[...].astype(f32)
        lane = jax.lax.broadcasted_iota(jnp.int32, (R, 128), 1)
        row = jax.lax.broadcasted_iota(jnp.int32, (R, 128), 0)
        even = (lane & 1) == 0
        low16 = (lane & 16) == 0
        scale = DH ** -0.5

        def layer(l, _):
            xn = _ln(xs[...]).astype(bf16)
            q = _dot(xn, wqkv[:, 0:D])
            for j in range(NB):
                qs[j] = q[:, j * 128:(j + 1) * 128]
            k = _dot(xn, wqkv[:, D:2 * D])
            for j in range(NB):
                ks[j, 0:HALO, :] = kh[l, j]
                ks[j, HALO:HALO + TM, :] = k[:, j * 128:(j + 1) * 128]
                kh[l, j] = k[TM - HALO:, j * 128:(j + 1) * 128]
            v = _dot(xn, wqkv[:, 2 * D:3 * D])
            for j in range(NB):
                vj = v[:, j * 128:(j + 1) * 128]
                vs[j, HALO:HALO + TM, :] = vj

                @pl.when(step == 0)
                def _():
                    vh[l, j] = jnp.broadcast_to(vs[j, HALO:HALO + 1, :], (HALO, 128))
                vs[j, 0:HALO, :] = vh[l, j]
                vh[l, j] = vj[TM - HALO:, :]

            for r0 in range(0, TM, R):
                t = [None] * W
                for j in range(NB):
                    qj = qs[j, r0:r0 + R, :]
                    for w in range(W):
                        p = qj * ks[j, pl.ds(HALO + r0 - DIL * w, R), :]
                        t[w] = p if t[w] is None else t[w] + p
                lg = []
                for w in range(W):
                    a = t[w]
                    a = a + jnp.where(even, pltpu.roll(a, 127, 1), pltpu.roll(a, 1, 1))
                    a = a + jnp.where(low16, pltpu.roll(a, 112, 1), pltpu.roll(a, 16, 1))
                    a = a * scale
                    if r0 < DIL * w:
                        a = jnp.where(step * TM + r0 + row - DIL * w >= 0, a, -1e9)
                    lg.append(a)
                mx = functools.reduce(jnp.maximum, lg)
                e = [jnp.exp(a - mx) for a in lg]
                den = functools.reduce(lambda a, b: a + b, e)
                inv = 1.0 / den
                pr = [a * inv for a in e]
                for j in range(NB):
                    acc = None
                    for w in range(W):
                        p = pr[w] * vs[j, pl.ds(HALO + r0 - DIL * w, R), :]
                        acc = p if acc is None else acc + p
                    os_[r0:r0 + R, j * 128:(j + 1) * 128] = acc.astype(bf16)

            x1 = xs[...] + _dot(os_[...], wo[...])
            xs[...] = x1
            os_[...] = _ln(x1).astype(bf16)

            def ffn(c, _):
                c0 = pl.multiple_of(c * FC, FC) if ffn_loop else c * FC
                xn2 = os_[...]
                g = _dot(xn2, w1[:, pl.ds(c0, FC)])
                u = _dot(xn2, w3[:, pl.ds(c0, FC)])
                h = (g * jax.nn.sigmoid(g) * u).astype(bf16)
                xs[...] += _dot(h, w2[pl.ds(c0, FC), :])
                return 0
            if ffn_loop:
                jax.lax.fori_loop(0, F // FC, ffn, 0)
            else:
                for c in range(F // FC):
                    ffn(c, 0)
            return 0

        if layer_loop:
            jax.lax.fori_loop(0, 2, layer, 0)
        else:
            layer(0, 0)
            layer(1, 0)
        o_ref[...] = xs[...].astype(bf16)

    @jax.jit
    def run(A_x, A_wqkv, A_wo, B_x, B_w1, B_w3, B_w2):
        x = A_x.reshape(S, D)
        any_spec = pl.BlockSpec(memory_space=pl.ANY)
        out = pl.pallas_call(
            kernel,
            grid=(S // TM,),
            in_specs=[pl.BlockSpec((TM, D), lambda i: (i, 0))] + [any_spec] * 5,
            out_specs=pl.BlockSpec((TM, D), lambda i: (i, 0)),
            out_shape=jax.ShapeDtypeStruct((S, D), bf16),
            scratch_shapes=[
                pltpu.VMEM((D, 3 * D), bf16), pltpu.VMEM((NB, D, 128), bf16), pltpu.VMEM((D, D), bf16),
                pltpu.VMEM((D, F), bf16), pltpu.VMEM((D, F), bf16), pltpu.VMEM((F, D), bf16),
                pltpu.VMEM((TM, D), f32),
                pltpu.VMEM((NB, TM, 128), f32),
                pltpu.VMEM((NB, HALO + TM, 128), f32), pltpu.VMEM((NB, HALO + TM, 128), f32),
                pltpu.VMEM((2, NB, HALO, 128), f32), pltpu.VMEM((2, NB, HALO, 128), f32),
                pltpu.VMEM((TM, D), bf16),
                pltpu.SemaphoreType.DMA((7,)),
            ],
            compiler_params=pltpu.CompilerParams(
                dimension_semantics=("arbitrary",), vmem_limit_bytes=100 * 1024 * 1024),
        )(x, A_wqkv, A_wo, B_w1, B_w3, B_w2)
        return out.reshape(1, S, D)
    return run


_run = make()


def pallas_interleave_layers__sliding_local_dilated__glu_gated_swiglu__prompt_kernel(A_x, A_wqkv, A_wo, B_x, B_w1, B_w3, B_w2):
    return _run(A_x, A_wqkv, A_wo, B_x, B_w1, B_w3, B_w2)
```

```python
import functools
import jax
import jax.numpy as jnp
import jax.experimental.pallas as pl
import jax.experimental.pallas.tpu as pltpu

S, D, F = 2048, 1024, 3584
H, DH, W, DIL = 32, 32, 8, 2
HALO = 16
NB = D // 128
FB = F // 128
f32, bf16 = jnp.float32, jnp.bfloat16
Q_, K_, V_, T_, X1_, X2_, XN_ = range(7)


def _ln(x):
    m = jnp.mean(x, axis=-1, keepdims=True)
    d = x - m
    v = jnp.mean(d * d, axis=-1, keepdims=True)
    return d * jax.lax.rsqrt(v + 1e-5)


def _dot(a, b):
    return jnp.dot(a, b, preferred_element_type=f32)


def _cols(ref, start, count, rows=slice(None)):
    return jnp.concatenate([ref[start + c, rows, :] for c in range(count)], axis=1)


def _swap_blocks(blocks, lane):
    blocks = list(blocks)
    for b in range(3):
        dist = 2 << b
        low = (lane & dist) == 0
        for c in range(NB):
            if c & (1 << b):
                continue
            A, B = blocks[c], blocks[c | (1 << b)]
            blocks[c] = jnp.where(low, A, pltpu.roll(B, dist, 1))
            blocks[c | (1 << b)] = jnp.where(low, pltpu.roll(A, 128 - dist, 1), B)
    return blocks


def make(RB=256, FC=14, KC=4, R=16, PR=256, LR=32, GQ=1, GV=1, NL=2, AU=2, DS=24, SP=1, L2=32, flags=None):
    NBLK = S // RB
    NJOB = NL * NBLK
    NG = FB // FC

    def kernel(x_hbm, wqkv_hbm, wo_hbm, w1_hbm, w3_hbm, w2_hbm, o_ref,
               wqkv, wo_raw, wo, w1, w3, w2, xb, xs, att, hb, sems):
        n = pl.program_id(0)
        zero = (n // 4096) * 8

        def pinned(r0, size):
            return pl.ds(pl.multiple_of(r0 + zero, 8), size)

        def rows(b):
            return pl.ds(pl.multiple_of(b * RB, RB), RB)

        def col_copies(src, dst, lo, hi, sem):
            return [pltpu.make_async_copy(src.at[:, pl.ds(c * 128, 128)], dst.at[c], sems.at[sem]) for c in range(lo, hi)]

        def row_copy(lo, hi, sem):
            return [pltpu.make_async_copy(x_hbm.at[pl.ds(lo, hi - lo)], xb.at[pl.ds(lo, hi - lo)], sems.at[sem])]

        cp_x0, cp_x1, cp_xr = row_copy(0, RB, 0), row_copy(RB, 2 * RB, 1), row_copy(2 * RB, S, 2)
        cp_qkv = [col_copies(wqkv_hbm, wqkv, i * NB, (i + 1) * NB, 3 + i) for i in range(3)]
        cp_wo = col_copies(wo_hbm, wo_raw, 0, NB, 6)
        cp_w2 = col_copies(w2_hbm, w2, 0, NB, 7)
        cp_gu = [col_copies(w1_hbm, w1, g * FC, (g + 1) * FC, 8 + g) + col_copies(w3_hbm, w3, g * FC, (g + 1) * FC, 8 + g)
                 for g in range(NG)]

        def start(cps):
            for c in cps:
                c.start()

        def wait(cps):
            for c in cps:
                c.wait()

        def permute_w(i):
            def body(r, _):
                lane = jax.lax.broadcasted_iota(jnp.int32, (PR // 2, 128), 1)
                rs = pl.ds(pl.multiple_of(r * PR, PR), PR)
                blocks = [pltpu.bitcast(wqkv[i * NB + c, rs, :], jnp.uint32) for c in range(NB)]
                blocks = _swap_blocks(blocks, lane)
                for c in range(NB):
                    wqkv[i * NB + c, rs, :] = pltpu.bitcast(blocks[c], bf16)
                return 0
            jax.lax.fori_loop(0, D // PR, body, 0)

        def permute_wo():
            src = wo_raw.bitcast(jnp.uint32)

            def body(c, _):
                for j in range(NB):
                    blk = jnp.concatenate([src[c, pl.ds(m * 8 + j, 8, stride=64), :] for m in range(8)], axis=0)
                    wo[c, pl.ds(j * 128, 128), :] = pltpu.bitcast(blk, bf16)
                return 0
            jax.lax.fori_loop(0, NB, body, 0)

        def ln_store(plane, r0, x):
            y = pltpu.bitcast(_ln(x).astype(bf16), f32)
            dst = pinned(r0 // 2, x.shape[0] // 2)
            for j in range(NB):
                att[plane, j, dst, :] = y[:, j * 128:(j + 1) * 128]

        def staged(plane, r0, size):
            return jnp.concatenate([att[plane, j, HALO + r0:HALO + r0 + size, :] for j in range(NB)], axis=1)

        def stage(plane, x):
            for j in range(NB):
                att[plane, j, HALO:HALO + RB, :] = x[:, j * 128:(j + 1) * 128]

        def ln_loop(plane, b):
            def body(i, _):
                r0 = pl.multiple_of(i * 128, 128)
                ln_store(plane, r0, xs[pl.ds(b * RB + r0, 128), :])
                return 0
            jax.lax.fori_loop(0, RB // 128, body, 0)

        def normed(plane):
            return jnp.concatenate([pltpu.bitcast(att[plane, j, 0:RB // 2, :], bf16) for j in range(NB)], axis=1)

        def proj(i, first):
            y = _dot(normed(X1_), _cols(wqkv, i * NB, NB))
            for j in range(NB):
                yj = y[:, j * 128:(j + 1) * 128]
                if i != Q_:
                    edge = jnp.broadcast_to(yj[0:1, :], (HALO, 128))
                    att[i, j, 0:HALO, :] = jnp.where(first, edge, att[i, j, RB:RB + HALO, :])
                att[i, j, HALO:HALO + RB, :] = yj

        def probs(r0, pos0, chain):
            here = pl.ds(HALO + r0, R)
            q = [att[Q_, j, here, :] for j in range(NB)]
            t = []
            for w in range(W):
                acc = None
                for j in range(NB):
                    p = q[j] * att[K_, j, pl.ds(HALO + r0 - DIL * w, R), :]
                    acc = p if acc is None else acc + p
                if chain and w % GQ == GQ - 1 and w < W - 1:
                    att[T_, w, pinned(HALO + r0, R), :] = acc
                    acc = None
                t.append(acc)
            t = [att[T_, w, here, :] if a is None else a for w, a in enumerate(t)]
            lane = jax.lax.broadcasted_iota(jnp.int32, (R, 128), 1)
            even = (lane & 1) == 0
            low16 = (lane & 16) == 0
            lg = []
            for w in range(W):
                a = t[w]
                a = a + jnp.where(even, pltpu.roll(a, 127, 1), pltpu.roll(a, 1, 1))
                a = a + jnp.where(low16, pltpu.roll(a, 112, 1), pltpu.roll(a, 16, 1))
                a = a * (DH ** -0.5)
                if not chain or r0 < DIL * w:
                    row = jax.lax.broadcasted_iota(jnp.int32, (R, 128), 0)
                    a = jnp.where(pos0 + r0 + row - DIL * w >= 0, a, -1e9)
                lg.append(a)
            mx = functools.reduce(jnp.maximum, lg)
            e = [jnp.exp(a - mx) for a in lg]
            inv = 1.0 / functools.reduce(lambda a, b: a + b, e)
            return [a * inv for a in e]

        def mix(r0, pr, chain):
            here = pl.ds(HALO + r0, R)
            for j in range(NB):
                acc = None
                for w in range(W):
                    p = pr[w] * att[V_, j, pl.ds(HALO + r0 - DIL * w, R), :]
                    acc = p if acc is None else acc + p
                att[Q_, j, pinned(HALO + r0, R) if chain and j % GV == GV - 1 else here, :] = acc

        def out_proj(b, keep):
            o = jnp.concatenate([att[Q_, j, HALO:HALO + RB, :].astype(bf16) for j in range(NB)], axis=1)
            x1 = xs[rows(b), :] + _dot(o, _cols(wo, 0, NB))
            xs[rows(b), :] = x1
            if keep:
                stage(Q_, x1)

        def gate_up(c0, fc):
            x2 = normed(X2_)
            g = _dot(x2, _cols(w1, c0, fc))
            u = _dot(x2, _cols(w3, c0, fc))
            h = (g * jax.nn.sigmoid(g) * u).astype(bf16)
            for c in range(fc):
                hb[c0 + c] = h[:, c * 128:(c + 1) * 128]

        def load_x(lo, hi):
            def body(i, _):
                rs = pl.ds(pl.multiple_of(i * 64, 64), 64)
                xs[rs, :] = xb[rs, :].astype(f32)
                return 0
            jax.lax.fori_loop(lo // 64, hi // 64, body, 0)

        blk = n % NBLK
        prev = jnp.maximum(n - 1, 0) % NBLK
        nxt = (n + 1) % NBLK

        @pl.when(n == 0)
        def _start():
            start(cp_x0 + cp_qkv[0] + cp_qkv[1])
            att[K_:V_ + 1, :, RB:RB + HALO, :] = jnp.zeros((2, NB, HALO, 128), f32)
            wait(cp_x0)
            load_x(0, RB)
            ln_loop(X1_, 0)
            for i in range(3):
                wait(cp_qkv[i])
                start([cp_qkv[2] + cp_x1, cp_wo + cp_xr, cp_gu[0]][i])
                permute_w(i)
            wait(cp_x1)
            load_x(RB, 2 * RB)

        @pl.when(n < NJOB)
        def _qkv():
            first = blk == 0
            stage(XN_, xs[rows(nxt), :])
            proj(Q_, first)
            proj(K_, first)
            proj(V_, first)

        @pl.when(n == 0)
        def _first():
            wait(cp_wo)
            start(sum(cp_gu[1:], []) + cp_w2)
            permute_wo()

            def body(i, _):
                r0 = pl.multiple_of(i * R, R)
                mix(r0, probs(r0, 0, False), False)
                return 0
            jax.lax.fori_loop(0, RB // R, body, 0, unroll=AU)
            out_proj(0, False)
            ln_loop(X2_, 0)
            ln_loop(X1_, 1)
            wait(cp_xr)
            load_x(2 * RB, S)

        @pl.when(n > 0)
        def _gate_up():
            def body(c, _):
                @pl.when(n == 1)
                def _():
                    for i in range(NG):
                        @pl.when(c == i)
                        def _():
                            wait(cp_gu[i])
                gate_up(c * FC, FC)
                return 0
            jax.lax.fori_loop(0, NG, body, 0)

        @pl.when(n == 1)
        def _wait_b():
            wait(cp_w2)

        @pl.when(jnp.logical_and(n > 0, n < NJOB))
        def _attn():
            pr = probs(0, blk * RB, True)
            for r0 in range(0, RB, R):
                if r0 % LR == 0:
                    x = staged(XN_, r0, LR)
                pr_next = probs(r0 + R, blk * RB, True) if r0 + R < RB and SP else None
                mix(r0, pr, True)
                if r0 % LR == 0:
                    ln_store(X1_, r0, x)
                pr = probs(r0 + R, blk * RB, True) if r0 + R < RB and not SP else pr_next
            xs[rows(prev), :] += _dot(_cols(hb, 0, DS), _cols(w2, 0, NB, slice(0, DS * 128)))
            out_proj(blk, True)
            x = staged(Q_, 0, L2)
            for r0 in range(0, RB, L2):
                x_next = staged(Q_, r0 + L2, L2) if r0 + L2 < RB else None
                ln_store(X2_, r0, x)
                x = x_next
            y = xs[rows(prev), :] + _dot(_cols(hb, DS, FB - DS), _cols(w2, 0, NB, slice(DS * 128, F)))
            xs[rows(prev), :] = y
            o_ref[...] = y.astype(bf16)

        @pl.when(n == NJOB)
        def _last():
            def body(c, _):
                cs = pl.ds(pl.multiple_of(c * KC * 128, KC * 128), KC * 128)
                xs[rows(prev), :] += _dot(_cols(hb, c * KC, KC), _cols(w2, 0, NB, cs))
                return 0
            jax.lax.fori_loop(0, FB // KC, body, 0)
            o_ref[...] = xs[rows(prev), :].astype(bf16)

    @jax.jit
    def run(A_x, A_wqkv, A_wo, B_x, B_w1, B_w3, B_w2):
        x = A_x.reshape(S, D)
        any_spec = pl.BlockSpec(memory_space=pl.ANY)
        out = pl.pallas_call(
            kernel,
            grid=(NJOB + 1,),
            in_specs=[any_spec] * 6,
            out_specs=pl.BlockSpec((RB, D), lambda i: (jnp.maximum(i - ((NL - 1) * NBLK + 1), 0), 0)),
            out_shape=jax.ShapeDtypeStruct((S, D), bf16),
            scratch_shapes=[
                pltpu.VMEM((3 * NB, D, 128), bf16), pltpu.VMEM((NB, D, 128), bf16), pltpu.VMEM((NB, D, 128), bf16),
                pltpu.VMEM((FB, D, 128), bf16), pltpu.VMEM((FB, D, 128), bf16), pltpu.VMEM((NB, F, 128), bf16),
                pltpu.VMEM((S, D), bf16), pltpu.VMEM((S, D), f32),
                pltpu.VMEM((7, NB, HALO + RB, 128), f32),
                pltpu.VMEM((FB, RB, 128), bf16),
                pltpu.SemaphoreType.DMA((8 + NG,)),
            ],
            compiler_params=pltpu.CompilerParams(
                dimension_semantics=("arbitrary",), vmem_limit_bytes=100 * 1024 * 1024, flags=flags),
        )(x, A_wqkv, A_wo, B_w1, B_w3, B_w2)
        return out.reshape(1, S, D)
    return run


_run = make(DS=24,SP=0)


def pallas_interleave_layers__sliding_local_dilated__glu_gated_swiglu__prompt_kernel(A_x, A_wqkv, A_wo, B_x, B_w1, B_w3, B_w2):
    return _run(A_x, A_wqkv, A_wo, B_x, B_w1, B_w3, B_w2)
```

```python
import functools
import jax
import jax.numpy as jnp
import jax.experimental.pallas as pl
import jax.experimental.pallas.tpu as pltpu

S, D, F = 2048, 1024, 3584
H, DH, W, DIL = 32, 32, 8, 2
HALO = 16
NB = D // 128
FB = F // 128
f32, bf16 = jnp.float32, jnp.bfloat16
Q_, K_, V_, T_, X1_, X2_, XN_ = range(7)
LOG2E = 1.4426950408889634


def _ln(x):
    m = jnp.mean(x, axis=-1, keepdims=True)
    d = x - m
    v = jnp.mean(d * d, axis=-1, keepdims=True)
    return d * jax.lax.rsqrt(v + 1e-5)


def _dot(a, b):
    return jnp.dot(a, b, preferred_element_type=f32)


def _cols(ref, start, count, rows=slice(None)):
    return jnp.concatenate([ref[start + c, rows, :] for c in range(count)], axis=1)


def _swap_blocks(blocks, lane):
    blocks = list(blocks)
    for b in range(3):
        dist = 2 << b
        low = (lane & dist) == 0
        for c in range(NB):
            if c & (1 << b):
                continue
            A, B = blocks[c], blocks[c | (1 << b)]
            blocks[c] = jnp.where(low, A, pltpu.roll(B, dist, 1))
            blocks[c | (1 << b)] = jnp.where(low, pltpu.roll(A, 128 - dist, 1), B)
    return blocks


def make(RB=256, FC=14, KC=4, R=16, PR=256, LR=32, GQ=1, GV=1, NL=2, AU=2, DS=24, SP=0, L2=32, CH=2, HQ=1, HV=1, flags=None):
    NBLK = S // RB
    NJOB = NL * NBLK
    NG = FB // FC

    def kernel(x_hbm, wqkv_hbm, wo_hbm, w1_hbm, w3_hbm, w2_hbm, o_ref,
               wq, wk, wv, wo_raw, wo, w1, w3, w2, xb, xs, att, hb, sems):
        n = pl.program_id(0)
        zero = (n // 4096) * 8

        def pinned(r0, size):
            return pl.ds(pl.multiple_of(r0 + zero, 8), size)

        def rows(b):
            return pl.ds(pl.multiple_of(b * RB, RB), RB)

        def col_copies(src, dst, lo, hi, sem):
            return [pltpu.make_async_copy(src.at[:, pl.ds(c * 128, 128)], dst.at[c], sems.at[sem]) for c in range(lo, hi)]

        def row_copy(lo, hi, sem):
            return [pltpu.make_async_copy(x_hbm.at[pl.ds(lo, hi - lo)], xb.at[pl.ds(lo, hi - lo)], sems.at[sem])]

        cp_x0, cp_x1, cp_xr = row_copy(0, RB, 0), row_copy(RB, 2 * RB, 1), row_copy(2 * RB, S, 2)
        wqkv = (wq, wk, wv)
        cp_q = [[pltpu.make_async_copy(wqkv_hbm.at[pl.ds(r * PR, PR), pl.ds(c * 128, 128)], wq.at[c, pl.ds(r * PR, PR)],
                                       sems.at[8 + NG + r]) for c in range(NB)] for r in range(D // PR)]
        cp_k, cp_v = [[pltpu.make_async_copy(wqkv_hbm.at[:, pl.ds(i * D + c * 128, 128)], wqkv[i].at[c], sems.at[3 + i])
                       for c in range(NB)] for i in (1, 2)]
        cp_wo = col_copies(wo_hbm, wo_raw, 0, NB, 6)
        cp_w2 = col_copies(w2_hbm, w2, 0, NB, 7)
        cp_gu = [col_copies(w1_hbm, w1, g * FC, (g + 1) * FC, 8 + g) + col_copies(w3_hbm, w3, g * FC, (g + 1) * FC, 8 + g)
                 for g in range(NG)]

        def start(cps):
            for c in cps:
                c.start()

        def wait(cps):
            for c in cps:
                c.wait()

        def permute_rows(w, r0, size):
            lane = jax.lax.broadcasted_iota(jnp.int32, (size // 2, 128), 1)
            rs = pl.ds(pl.multiple_of(r0, size), size)
            blocks = _swap_blocks([pltpu.bitcast(w[c, rs, :], jnp.uint32) for c in range(NB)], lane)
            for c in range(NB):
                w[c, rs, :] = pltpu.bitcast(blocks[c], bf16)

        def permute_wo():
            src = wo_raw.bitcast(jnp.uint32)

            def body(c, _):
                for j in range(NB):
                    blk = jnp.concatenate([src[c, pl.ds(m * 8 + j, 8, stride=64), :] for m in range(8)], axis=0)
                    wo[c, pl.ds(j * 128, 128), :] = pltpu.bitcast(blk, bf16)
                return 0
            jax.lax.fori_loop(0, NB, body, 0)

        def ln_store(plane, r0, x):
            y = pltpu.bitcast(_ln(x).astype(bf16), f32)
            dst = pinned(r0 // 2, x.shape[0] // 2)
            for j in range(NB):
                att[plane, j, dst, :] = y[:, j * 128:(j + 1) * 128]

        def staged(plane, r0, size):
            return jnp.concatenate([att[plane, j, HALO + r0:HALO + r0 + size, :] for j in range(NB)], axis=1)

        def stage(plane, x):
            for j in range(NB):
                att[plane, j, HALO:HALO + RB, :] = x[:, j * 128:(j + 1) * 128]

        def ln_loop(plane, b):
            def body(i, _):
                r0 = pl.multiple_of(i * 128, 128)
                ln_store(plane, r0, xs[pl.ds(b * RB + r0, 128), :])
                return 0
            jax.lax.fori_loop(0, RB // 128, body, 0)

        def normed(plane):
            return jnp.concatenate([pltpu.bitcast(att[plane, j, 0:RB // 2, :], bf16) for j in range(NB)], axis=1)

        def proj(i, first, j0=0, nj=NB):
            y = _dot(normed(X1_), _cols(wqkv[i], j0, nj))
            for j in range(nj):
                yj = y[:, j * 128:(j + 1) * 128]
                if i != Q_:
                    edge = jnp.broadcast_to(yj[0:1, :], (HALO, 128))
                    if first is not True:
                        edge = jnp.where(first, edge, att[i, j0 + j, RB:RB + HALO, :])
                    att[i, j0 + j, 0:HALO, :] = edge
                att[i, j0 + j, HALO:HALO + RB, :] = yj

        def probs(r0, pos0, chain):
            here = pl.ds(HALO + r0, R)
            q = [att[Q_, j, here, :] for j in range(NB)]
            t = []
            for w in range(W):
                acc = None
                for j in range(NB):
                    p = q[j] * att[K_, j, pl.ds(HALO + r0 - DIL * w, R), :]
                    acc = p if acc is None else acc + p
                    if chain and HQ == 2 and j == NB // 2 - 1:
                        att[T_, w, pinned(HALO + r0, R), :] = acc
                if chain and w % GQ == GQ - 1 and w < W - 1:
                    att[T_, w, pinned(HALO + r0, R), :] = acc
                    acc = None
                t.append(acc)
            t = [att[T_, w, here, :] if a is None else a for w, a in enumerate(t)]
            lane = jax.lax.broadcasted_iota(jnp.int32, (R, 128), 1)
            even = (lane & 1) == 0
            low16 = (lane & 16) == 0
            lg = []
            for w in range(W):
                a = t[w]
                a = a + jnp.where(even, pltpu.roll(a, 127, 1), pltpu.roll(a, 1, 1))
                a = a + jnp.where(low16, pltpu.roll(a, 112, 1), pltpu.roll(a, 16, 1))
                a = a * (DH ** -0.5 * LOG2E)
                if not chain or r0 < DIL * w:
                    row = jax.lax.broadcasted_iota(jnp.int32, (R, 128), 0)
                    a = jnp.where(pos0 + r0 + row - DIL * w >= 0, a, -1e9 * LOG2E)
                lg.append(a)
            mx = functools.reduce(jnp.maximum, lg)
            e = [jnp.exp2(a - mx) for a in lg]
            inv = 1.0 / functools.reduce(lambda a, b: a + b, e)
            return [a * inv for a in e]

        def mix(r0, pr, chain):
            here = pl.ds(HALO + r0, R)
            for j in range(NB):
                acc = None
                for w in range(W):
                    p = pr[w] * att[V_, j, pl.ds(HALO + r0 - DIL * w, R), :]
                    acc = p if acc is None else acc + p
                    if chain and HV == 2 and w == W // 2 - 1:
                        att[T_, j, pinned(HALO + r0, R), :] = acc
                att[Q_, j, pinned(HALO + r0, R) if chain and j % GV == GV - 1 else here, :] = acc

        def out_proj(b, keep):
            o = jnp.concatenate([att[Q_, j, HALO:HALO + RB, :].astype(bf16) for j in range(NB)], axis=1)
            x1 = xs[rows(b), :] + _dot(o, _cols(wo, 0, NB))
            xs[rows(b), :] = x1
            if keep:
                stage(Q_, x1)

        def gate_up(c0, fc):
            x2 = normed(X2_)
            g = _dot(x2, _cols(w1, c0, fc))
            u = _dot(x2, _cols(w3, c0, fc))
            h = (g * jax.nn.sigmoid(g) * u).astype(bf16)
            for c in range(fc):
                hb[c0 + c] = pltpu.bitcast(h[:, c * 128:(c + 1) * 128], f32)

        def hidden(c0, nc):
            return jnp.concatenate([pltpu.bitcast(hb[c0 + c], bf16) for c in range(nc)], axis=1)

        def load_x(lo, hi):
            def body(i, _):
                rs = pl.ds(pl.multiple_of(i * 64, 64), 64)
                xs[rs, :] = xb[rs, :].astype(f32)
                return 0
            jax.lax.fori_loop(lo // 64, hi // 64, body, 0)

        blk = n % NBLK
        prev = jnp.maximum(n - 1, 0) % NBLK
        nxt = (n + 1) % NBLK

        @pl.when(n == 0)
        def _start():
            start(cp_x0 + sum(cp_q, []))
            wait(cp_x0)
            load_x(0, RB)
            ln_loop(X1_, 0)
            start(cp_k)

            def body(r, _):
                for i in range(D // PR):
                    @pl.when(r == i)
                    def _():
                        wait(cp_q[i])
                permute_rows(wq, r * PR, PR)
                return 0
            jax.lax.fori_loop(0, D // PR, body, 0)
            for i in range(3):
                if i < 2:
                    wait((cp_k, cp_v)[i])
                start((cp_v + cp_x1, cp_wo + cp_xr, cp_gu[0])[i])

                def body(c, _, i=i):
                    proj(i, True, c * (NB // CH), NB // CH)
                    if i < 2:
                        permute_rows(wqkv[i + 1], c * (D // CH), D // CH)
                    return 0
                jax.lax.fori_loop(0, CH, body, 0)
            wait(cp_x1)
            load_x(RB, 2 * RB)

        @pl.when(jnp.logical_and(n > 0, n < NJOB))
        def _qkv():
            first = blk == 0
            stage(XN_, xs[rows(nxt), :])
            proj(Q_, first)
            proj(K_, first)
            proj(V_, first)

        @pl.when(n == 0)
        def _first():
            wait(cp_wo)
            start(sum(cp_gu[1:], []) + cp_w2)
            permute_wo()

            def body(i, _):
                r0 = pl.multiple_of(i * R, R)
                mix(r0, probs(r0, 0, False), False)
                return 0
            jax.lax.fori_loop(0, RB // R, body, 0, unroll=AU)
            out_proj(0, False)
            ln_loop(X2_, 0)
            ln_loop(X1_, 1)
            wait(cp_xr)
            load_x(2 * RB, S)

        @pl.when(n > 0)
        def _gate_up():
            def body(c, _):
                @pl.when(n == 1)
                def _():
                    for i in range(NG):
                        @pl.when(c == i)
                        def _():
                            wait(cp_gu[i])
                gate_up(c * FC, FC)
                return 0
            jax.lax.fori_loop(0, NG, body, 0)

        @pl.when(n == 1)
        def _wait_b():
            wait(cp_w2)

        @pl.when(jnp.logical_and(n > 0, n < NJOB))
        def _attn():
            pr = probs(0, blk * RB, True)
            for r0 in range(0, RB, R):
                if r0 % LR == 0:
                    x = staged(XN_, r0, LR)
                pr_next = probs(r0 + R, blk * RB, True) if r0 + R < RB and SP else None
                mix(r0, pr, True)
                if r0 % LR == 0:
                    ln_store(X1_, r0, x)
                pr = probs(r0 + R, blk * RB, True) if r0 + R < RB and not SP else pr_next
            xs[rows(prev), :] += _dot(hidden(0, DS), _cols(w2, 0, NB, slice(0, DS * 128)))
            out_proj(blk, True)
            x = staged(Q_, 0, L2)
            for r0 in range(0, RB, L2):
                x_next = staged(Q_, r0 + L2, L2) if r0 + L2 < RB else None
                ln_store(X2_, r0, x)
                x = x_next
            y = xs[rows(prev), :] + _dot(hidden(DS, FB - DS), _cols(w2, 0, NB, slice(DS * 128, F)))
            xs[rows(prev), :] = y
            o_ref[...] = y.astype(bf16)

        @pl.when(n == NJOB)
        def _last():
            def body(c, _):
                cs = pl.ds(pl.multiple_of(c * KC * 128, KC * 128), KC * 128)
                xs[rows(prev), :] += _dot(hidden(c * KC, KC), _cols(w2, 0, NB, cs))
                return 0
            jax.lax.fori_loop(0, FB // KC, body, 0)
            o_ref[...] = xs[rows(prev), :].astype(bf16)

    @jax.jit
    def run(A_x, A_wqkv, A_wo, B_x, B_w1, B_w3, B_w2):
        x = A_x.reshape(S, D)
        any_spec = pl.BlockSpec(memory_space=pl.ANY)
        out = pl.pallas_call(
            kernel,
            grid=(NJOB + 1,),
            in_specs=[any_spec] * 6,
            out_specs=pl.BlockSpec((RB, D), lambda i: (jnp.maximum(i - ((NL - 1) * NBLK + 1), 0), 0)),
            out_shape=jax.ShapeDtypeStruct((S, D), bf16),
            scratch_shapes=[
                *[pltpu.VMEM((NB, D, 128), bf16)] * 5,
                pltpu.VMEM((FB, D, 128), bf16), pltpu.VMEM((FB, D, 128), bf16), pltpu.VMEM((NB, F, 128), bf16),
                pltpu.VMEM((S, D), bf16), pltpu.VMEM((S, D), f32),
                pltpu.VMEM((7, NB, HALO + RB, 128), f32),
                pltpu.VMEM((FB, RB // 2, 128), f32),
                pltpu.SemaphoreType.DMA((8 + NG + D // PR,)),
            ],
            compiler_params=pltpu.CompilerParams(
                dimension_semantics=("arbitrary",), vmem_limit_bytes=100 * 1024 * 1024, flags=flags),
        )(x, A_wqkv, A_wo, B_w1, B_w3, B_w2)
        return out.reshape(1, S, D)
    return run


_run = make()


def pallas_interleave_layers__sliding_local_dilated__glu_gated_swiglu__prompt_kernel(A_x, A_wqkv, A_wo, B_x, B_w1, B_w3, B_w2):
    return _run(A_x, A_wqkv, A_wo, B_x, B_w1, B_w3, B_w2)
```

```python
import functools
import jax
import jax.numpy as jnp
import jax.experimental.pallas as pl
import jax.experimental.pallas.tpu as pltpu

S, D, F = 2048, 1024, 3584
H, DH, W, DIL = 32, 32, 8, 2
HALO = 16
NB = D // 128
FB = F // 128
f32, bf16 = jnp.float32, jnp.bfloat16
Q_, K_, V_, T_, X1_, X2_, XN_ = range(7)
LOG2E = 1.4426950408889634


def _ln(x):
    m = jnp.mean(x, axis=-1, keepdims=True)
    d = x - m
    v = jnp.mean(d * d, axis=-1, keepdims=True)
    return d * jax.lax.rsqrt(v + 1e-5)


def _dot(a, b):
    return jnp.dot(a, b, preferred_element_type=f32)


def _cols(ref, start, count, rows=slice(None)):
    return jnp.concatenate([ref[start + c, rows, :] for c in range(count)], axis=1)


def _swap_blocks(blocks, axis, unit):
    blocks = list(blocks)
    size = blocks[0].shape[axis]
    pos = jax.lax.broadcasted_iota(jnp.int32, blocks[0].shape, axis)
    for b in range(3):
        dist = unit << b
        low = (pos & dist) == 0
        for c in range(NB):
            if c & (1 << b):
                continue
            A, B = blocks[c], blocks[c | (1 << b)]
            blocks[c] = jnp.where(low, A, pltpu.roll(B, dist, axis))
            blocks[c | (1 << b)] = jnp.where(low, pltpu.roll(A, size - dist, axis), B)
    return blocks


def make(RB=256, FC=14, KC=4, R=16, PR=256, LR=32, GQ=1, GV=1, NL=2, R0=32, DS=24, SP=0, L2=32, CH=2, HQ=1, HV=1, flags=None):
    NBLK = S // RB
    NJOB = NL * NBLK
    NG = FB // FC

    def kernel(x_hbm, wqkv_hbm, wo_hbm, w1_hbm, w3_hbm, w2_hbm, o_ref,
               wq, wk, wv, wo, w1, w3, w2, xb, xs, att, hb, sems):
        n = pl.program_id(0)
        zero = (n // 4096) * 8

        def pinned(r0, size):
            return pl.ds(pl.multiple_of(r0 + zero, 8), size)

        def rows(b):
            return pl.ds(pl.multiple_of(b * RB, RB), RB)

        def col_copies(src, dst, lo, hi, sem):
            return [pltpu.make_async_copy(src.at[:, pl.ds(c * 128, 128)], dst.at[c], sems.at[sem]) for c in range(lo, hi)]

        def row_copy(lo, hi, sem):
            return [pltpu.make_async_copy(x_hbm.at[pl.ds(lo, hi - lo)], xb.at[pl.ds(lo, hi - lo)], sems.at[sem])]

        cp_x0, cp_x1, cp_xr = row_copy(0, RB, 0), row_copy(RB, 3 * RB, 1), row_copy(3 * RB, S, 2)
        wqkv = (wq, wk, wv)
        def slab_copies(i, size, sem):
            return [[pltpu.make_async_copy(wqkv_hbm.at[pl.ds(r * size, size), pl.ds(i * D + c * 128, 128)],
                                           wqkv[i].at[c, pl.ds(r * size, size)], sems.at[sem + r])
                     for c in range(NB)] for r in range(D // size)]

        cp_q = slab_copies(Q_, PR, 8 + NG)
        cp_kv = [slab_copies(i, D // CH, 8 + NG + D // PR + (i - 1) * CH) for i in (K_, V_)]
        cp_wo = col_copies(wo_hbm, wo, 0, NB, 6)
        cp_w2 = col_copies(w2_hbm, w2, 0, NB, 7)
        cp_gu = [col_copies(w1_hbm, w1, g * FC, (g + 1) * FC, 8 + g) + col_copies(w3_hbm, w3, g * FC, (g + 1) * FC, 8 + g)
                 for g in range(NG)]

        def start(cps):
            for c in cps:
                c.start()

        def wait(cps):
            for c in cps:
                c.wait()

        def wait_one(groups, k):
            for i, cps in enumerate(groups):
                pl.when(k == i)(functools.partial(wait, cps))

        def permute_rows(w, r0, size):
            rs = pl.ds(pl.multiple_of(r0, size), size)
            blocks = _swap_blocks([pltpu.bitcast(w[c, rs, :], jnp.uint32) for c in range(NB)], 1, 2)
            for c in range(NB):
                w[c, rs, :] = pltpu.bitcast(blocks[c], bf16)

        def permute_wo():
            def body(m, _):
                rs = [pl.ds(pl.multiple_of(c * 128 + m * 16, 16), 16) for c in range(NB)]
                blocks = _swap_blocks([pltpu.bitcast(_cols(wo, 0, NB, r), jnp.uint32) for r in rs], 0, 1)
                for r, blk16 in zip(rs, blocks):
                    y = pltpu.bitcast(blk16, bf16)
                    for j in range(NB):
                        wo[j, r, :] = y[:, j * 128:(j + 1) * 128]
                return 0
            jax.lax.fori_loop(0, 8, body, 0)

        def ln_store(plane, r0, x):
            y = pltpu.bitcast(_ln(x).astype(bf16), f32)
            dst = pinned(r0 // 2, x.shape[0] // 2)
            for j in range(NB):
                att[plane, j, dst, :] = y[:, j * 128:(j + 1) * 128]

        def staged(plane, r0, size):
            return jnp.concatenate([att[plane, j, HALO + r0:HALO + r0 + size, :] for j in range(NB)], axis=1)

        def stage(plane, x):
            for j in range(NB):
                att[plane, j, HALO:HALO + RB, :] = x[:, j * 128:(j + 1) * 128]

        def ln_loop(plane, b):
            def body(i, _):
                r0 = pl.multiple_of(i * 128, 128)
                ln_store(plane, r0, xs[pl.ds(b * RB + r0, 128), :])
                return 0
            jax.lax.fori_loop(0, RB // 128, body, 0)

        def normed(plane):
            return jnp.concatenate([pltpu.bitcast(att[plane, j, 0:RB // 2, :], bf16) for j in range(NB)], axis=1)

        def proj(i, first, j0=0, nj=NB):
            y = _dot(normed(X1_), _cols(wqkv[i], j0, nj))
            for j in range(nj):
                yj = y[:, j * 128:(j + 1) * 128]
                if i != Q_:
                    edge = jnp.broadcast_to(yj[0:1, :], (HALO, 128))
                    if first is not True:
                        edge = jnp.where(first, edge, att[i, j0 + j, RB:RB + HALO, :])
                    att[i, j0 + j, 0:HALO, :] = edge
                att[i, j0 + j, HALO:HALO + RB, :] = yj

        def probs(r0, pos0, chain, R=R):
            here = pl.ds(HALO + r0, R)
            q = [att[Q_, j, here, :] for j in range(NB)]
            t = []
            for w in range(W):
                acc = None
                for j in range(NB):
                    p = q[j] * att[K_, j, pl.ds(HALO + r0 - DIL * w, R), :]
                    acc = p if acc is None else acc + p
                    if chain and HQ == 2 and j == NB // 2 - 1:
                        att[T_, w, pinned(HALO + r0, R), :] = acc
                if chain and w % GQ == GQ - 1 and w < W - 1:
                    att[T_, w, pinned(HALO + r0, R), :] = acc
                    acc = None
                t.append(acc)
            t = [att[T_, w, here, :] if a is None else a for w, a in enumerate(t)]
            lane = jax.lax.broadcasted_iota(jnp.int32, (R, 128), 1)
            even = (lane & 1) == 0
            low16 = (lane & 16) == 0
            lg = []
            for w in range(W):
                a = t[w]
                a = a + jnp.where(even, pltpu.roll(a, 127, 1), pltpu.roll(a, 1, 1))
                a = a + jnp.where(low16, pltpu.roll(a, 112, 1), pltpu.roll(a, 16, 1))
                a = a * (DH ** -0.5 * LOG2E)
                if not chain or r0 < DIL * w:
                    row = jax.lax.broadcasted_iota(jnp.int32, (R, 128), 0)
                    a = jnp.where(pos0 + r0 + row - DIL * w >= 0, a, -1e9 * LOG2E)
                lg.append(a)
            mx = functools.reduce(jnp.maximum, lg)
            e = [jnp.exp2(a - mx) for a in lg]
            inv = 1.0 / functools.reduce(lambda a, b: a + b, e)
            return [a * inv for a in e]

        def mix(r0, pr, chain, R=R):
            here = pl.ds(HALO + r0, R)
            for j in range(NB):
                acc = None
                for w in range(W):
                    p = pr[w] * att[V_, j, pl.ds(HALO + r0 - DIL * w, R), :]
                    acc = p if acc is None else acc + p
                    if chain and HV == 2 and w == W // 2 - 1:
                        att[T_, j, pinned(HALO + r0, R), :] = acc
                att[Q_, j, pinned(HALO + r0, R) if chain and j % GV == GV - 1 else here, :] = acc

        def out_proj(b, keep):
            o = jnp.concatenate([att[Q_, j, HALO:HALO + RB, :].astype(bf16) for j in range(NB)], axis=1)
            x1 = xs[rows(b), :] + _dot(o, _cols(wo, 0, NB))
            xs[rows(b), :] = x1
            if keep:
                stage(Q_, x1)

        def gate_up(c0, fc):
            x2 = normed(X2_)
            g = _dot(x2, _cols(w1, c0, fc))
            u = _dot(x2, _cols(w3, c0, fc))
            h = (g * jax.nn.sigmoid(g) * u).astype(bf16)
            for c in range(fc):
                hb[c0 + c] = pltpu.bitcast(h[:, c * 128:(c + 1) * 128], f32)

        def hidden(c0, nc):
            return jnp.concatenate([pltpu.bitcast(hb[c0 + c], bf16) for c in range(nc)], axis=1)

        def load_x(lo, hi):
            def body(i, _):
                rs = pl.ds(pl.multiple_of(i * 64, 64), 64)
                xs[rs, :] = xb[rs, :].astype(f32)
                return 0
            jax.lax.fori_loop(lo // 64, hi // 64, body, 0)

        blk = n % NBLK
        prev = jnp.maximum(n - 1, 0) % NBLK
        nxt = (n + 1) % NBLK

        @pl.when(n == 0)
        def _start():
            start(cp_x0 + sum(cp_q, []))
            wait(cp_x0)
            load_x(0, RB)
            ln_loop(X1_, 0)
            start(sum(cp_kv[0] + cp_kv[1], []))

            def body(r, _):
                wait_one(cp_q, r)
                permute_rows(wq, r * PR, PR)
                return 0
            jax.lax.fori_loop(0, D // PR, body, 0)
            for i in range(3):
                start((cp_x1 + cp_wo, cp_gu[0], cp_gu[1])[i])

                def body(c, _, i=i):
                    if i < 2:
                        wait_one(cp_kv[i], c)
                    proj(i, True, c * (NB // CH), NB // CH)
                    if i < 2:
                        permute_rows(wqkv[i + 1], c * (D // CH), D // CH)
                    return 0
                jax.lax.fori_loop(0, CH, body, 0)
            wait(cp_x1)
            load_x(RB, 3 * RB)

            wait(cp_wo)
            permute_wo()

            def body(i, _):
                r0 = pl.multiple_of(i * R0, R0)
                mix(r0, probs(r0, 0, False, R0), False, R0)
                return 0
            jax.lax.fori_loop(0, RB // R0, body, 0)
            start(cp_w2 + cp_xr)
            out_proj(0, False)
            ln_loop(X2_, 0)
            ln_loop(X1_, 1)

        @pl.when(n > 0)
        def _gate_up():
            def body(c, _):
                pl.when(n == 1)(lambda: wait_one(cp_gu, c))
                gate_up(c * FC, FC)
                return 0
            jax.lax.fori_loop(0, NG, body, 0)

        @pl.when(n == 1)
        def _wait_b():
            wait(cp_w2)

        @pl.when(n == 2)
        def _wait_x():
            wait(cp_xr)
            load_x(3 * RB, S)

        @pl.when(jnp.logical_and(n > 0, n < NJOB))
        def _attn():
            first = blk == 0
            stage(XN_, xs[rows(nxt), :])
            proj(Q_, first)
            proj(K_, first)
            proj(V_, first)
            pr = probs(0, blk * RB, True)
            for r0 in range(0, RB, R):
                if r0 % LR == 0:
                    x = staged(XN_, r0, LR)
                pr_next = probs(r0 + R, blk * RB, True) if r0 + R < RB and SP else None
                mix(r0, pr, True)
                if r0 % LR == 0:
                    ln_store(X1_, r0, x)
                pr = probs(r0 + R, blk * RB, True) if r0 + R < RB and not SP else pr_next
            xs[rows(prev), :] += _dot(hidden(0, DS), _cols(w2, 0, NB, slice(0, DS * 128)))
            out_proj(blk, True)
            x = staged(Q_, 0, L2)
            for r0 in range(0, RB, L2):
                x_next = staged(Q_, r0 + L2, L2) if r0 + L2 < RB else None
                ln_store(X2_, r0, x)
                x = x_next
            y = xs[rows(prev), :] + _dot(hidden(DS, FB - DS), _cols(w2, 0, NB, slice(DS * 128, F)))
            xs[rows(prev), :] = y
            o_ref[...] = y.astype(bf16)

        @pl.when(n == NJOB)
        def _last():
            def body(c, _):
                cs = pl.ds(pl.multiple_of(c * KC * 128, KC * 128), KC * 128)
                xs[rows(prev), :] += _dot(hidden(c * KC, KC), _cols(w2, 0, NB, cs))
                return 0
            jax.lax.fori_loop(0, FB // KC, body, 0)
            o_ref[...] = xs[rows(prev), :].astype(bf16)

    @jax.jit
    def run(A_x, A_wqkv, A_wo, B_x, B_w1, B_w3, B_w2):
        x = A_x.reshape(S, D)
        any_spec = pl.BlockSpec(memory_space=pl.ANY)
        out = pl.pallas_call(
            kernel,
            grid=(NJOB + 1,),
            in_specs=[any_spec] * 6,
            out_specs=pl.BlockSpec((RB, D), lambda i: (jnp.maximum(i - ((NL - 1) * NBLK + 1), 0), 0)),
            out_shape=jax.ShapeDtypeStruct((S, D), bf16),
            scratch_shapes=[
                *[pltpu.VMEM((NB, D, 128), bf16)] * 4,
                pltpu.VMEM((FB, D, 128), bf16), pltpu.VMEM((FB, D, 128), bf16), pltpu.VMEM((NB, F, 128), bf16),
                pltpu.VMEM((S, D), bf16), pltpu.VMEM((S, D), f32),
                pltpu.VMEM((7, NB, HALO + RB, 128), f32),
                pltpu.VMEM((FB, RB // 2, 128), f32),
                pltpu.SemaphoreType.DMA((8 + NG + D // PR + 2 * CH,)),
            ],
            compiler_params=pltpu.CompilerParams(
                dimension_semantics=("arbitrary",), vmem_limit_bytes=100 * 1024 * 1024, flags=flags),
        )(x, A_wqkv, A_wo, B_w1, B_w3, B_w2)
        return out.reshape(1, S, D)
    return run


_run = make()


def pallas_interleave_layers__sliding_local_dilated__glu_gated_swiglu__prompt_kernel(A_x, A_wqkv, A_wo, B_x, B_w1, B_w3, B_w2):
    return _run(A_x, A_wqkv, A_wo, B_x, B_w1, B_w3, B_w2)
```

```python
import functools
import jax
import jax.numpy as jnp
import jax.experimental.pallas as pl
import jax.experimental.pallas.tpu as pltpu

S, D, F = 2048, 1024, 3584
H, DH, W, DIL = 32, 32, 8, 2
HALO = 16
NB = D // 128
FB = F // 128
f32, bf16 = jnp.float32, jnp.bfloat16
Q_, K_, V_, T_, X1_, X2_, XN_, O_ = range(8)
LOG2E = 1.4426950408889634


def _ln(x):
    m = jnp.mean(x, axis=-1, keepdims=True)
    d = x - m
    v = jnp.mean(d * d, axis=-1, keepdims=True)
    return d * jax.lax.rsqrt(v + 1e-5)


def _dot(a, b):
    return jnp.dot(a, b, preferred_element_type=f32)


def _cols(ref, start, count, rows=slice(None)):
    return jnp.concatenate([ref[start + c, rows, :] for c in range(count)], axis=1)


def _swap_blocks(blocks, axis, unit):
    blocks = list(blocks)
    size = blocks[0].shape[axis]
    pos = jax.lax.broadcasted_iota(jnp.int32, blocks[0].shape, axis)
    for b in range(3):
        dist = unit << b
        low = (pos & dist) == 0
        for c in range(NB):
            if c & (1 << b):
                continue
            A, B = blocks[c], blocks[c | (1 << b)]
            blocks[c] = jnp.where(low, A, pltpu.roll(B, dist, axis))
            blocks[c | (1 << b)] = jnp.where(low, pltpu.roll(A, size - dist, axis), B)
    return blocks


def make(RB=256, FC=14, KC=4, R=16, PR=256, LR=32, GQ=1, GV=1, NL=2, R0=32, DS=25, SP=0, L2=32, CH=2, HQ=1, HV=1, LM=True, flags=None):
    NBLK = S // RB
    NJOB = NL * NBLK
    NG = FB // FC

    def kernel(x_hbm, wqkv_hbm, wo_hbm, w1_hbm, w3_hbm, w2_hbm, o_ref,
               wq, wk, wv, wo, w1, w3, w2, xb, xs, att, hb, sems):
        n = pl.program_id(0)
        zero = (n // 4096) * 8

        def pinned(r0, size):
            return pl.ds(pl.multiple_of(r0 + zero, 8), size)

        def rows(b):
            if isinstance(b, int):
                return slice(b * RB, (b + 1) * RB)
            return pl.ds(pl.multiple_of(b * RB, RB), RB)

        def col_copies(src, dst, lo, hi, sem):
            return [pltpu.make_async_copy(src.at[:, pl.ds(c * 128, 128)], dst.at[c], sems.at[sem]) for c in range(lo, hi)]

        def row_copy(lo, hi, sem):
            return [pltpu.make_async_copy(x_hbm.at[pl.ds(lo, hi - lo)], xb.at[pl.ds(lo, hi - lo)], sems.at[sem])]

        cp_x0, cp_x1, cp_x2, cp_xr = row_copy(0, RB, 0), row_copy(RB, 2 * RB, 1), row_copy(2 * RB, 3 * RB, 3), row_copy(3 * RB, S, 2)
        wqkv = (wq, wk, wv)
        def slab_copies(i, size, sem):
            return [[pltpu.make_async_copy(wqkv_hbm.at[pl.ds(r * size, size), pl.ds(i * D + c * 128, 128)],
                                           wqkv[i].at[c, pl.ds(r * size, size)], sems.at[sem + r])
                     for c in range(NB)] for r in range(D // size)]

        cp_q = slab_copies(Q_, PR, 8 + NG)
        cp_kv = [slab_copies(i, D // CH, 8 + NG + D // PR + (i - 1) * CH) for i in (K_, V_)]
        cp_wo = col_copies(wo_hbm, wo, 0, NB, 6)
        cp_w2 = col_copies(w2_hbm, w2, 0, NB, 7)
        cp_gu = [col_copies(w1_hbm, w1, g * FC, (g + 1) * FC, 8 + g) + col_copies(w3_hbm, w3, g * FC, (g + 1) * FC, 8 + g)
                 for g in range(NG)]

        def start(cps):
            for c in cps:
                c.start()

        def wait(cps):
            for c in cps:
                c.wait()

        def wait_one(groups, k):
            for i, cps in enumerate(groups):
                pl.when(k == i)(functools.partial(wait, cps))

        def permute_rows(w, r0, size):
            rs = pl.ds(pl.multiple_of(r0, size), size)
            blocks = _swap_blocks([pltpu.bitcast(w[c, rs, :], jnp.uint32) for c in range(NB)], 1, 2)
            for c in range(NB):
                w[c, rs, :] = pltpu.bitcast(blocks[c], bf16)

        def permute_wo():
            def body(m, _):
                rs = [pl.ds(pl.multiple_of(c * 128 + m * 16, 16), 16) for c in range(NB)]
                blocks = _swap_blocks([pltpu.bitcast(_cols(wo, 0, NB, r), jnp.uint32) for r in rs], 0, 1)
                for r, blk16 in zip(rs, blocks):
                    y = pltpu.bitcast(blk16, bf16)
                    for j in range(NB):
                        wo[j, r, :] = y[:, j * 128:(j + 1) * 128]
                return 0
            jax.lax.fori_loop(0, 8, body, 0)

        def ln_store(plane, r0, x):
            y = pltpu.bitcast(_ln(x).astype(bf16), f32)
            dst = pinned(r0 // 2, x.shape[0] // 2)
            for j in range(NB):
                att[plane, j, dst, :] = y[:, j * 128:(j + 1) * 128]

        def staged(plane, r0, size):
            return jnp.concatenate([att[plane, j, HALO + r0:HALO + r0 + size, :] for j in range(NB)], axis=1)

        def stage(plane, x):
            for j in range(NB):
                att[plane, j, HALO:HALO + RB, :] = x[:, j * 128:(j + 1) * 128]

        def ln_loop(plane, b):
            def body(i, _):
                r0 = pl.multiple_of(i * 128, 128)
                ln_store(plane, r0, xs[pl.ds(b * RB + r0, 128), :])
                return 0
            jax.lax.fori_loop(0, RB // 128, body, 0)

        def normed(plane):
            return jnp.concatenate([pltpu.bitcast(att[plane, j, 0:RB // 2, :], bf16) for j in range(NB)], axis=1)

        def proj(i, first, j0=0, nj=NB):
            y = _dot(normed(X1_), _cols(wqkv[i], j0, nj))
            for j in range(nj):
                yj = y[:, j * 128:(j + 1) * 128]
                if i != Q_:
                    edge = jnp.broadcast_to(yj[0:1, :], (HALO, 128))
                    if first is not True:
                        edge = jnp.where(first, edge, att[i, j0 + j, RB:RB + HALO, :])
                    att[i, j0 + j, 0:HALO, :] = edge
                att[i, j0 + j, HALO:HALO + RB, :] = yj

        def probs(r0, pos0, chain, R=R):
            here = pl.ds(HALO + r0, R)
            q = [att[Q_, j, here, :] for j in range(NB)]
            t = []
            for w in range(W):
                acc = None
                for j in range(NB):
                    p = q[j] * att[K_, j, pl.ds(HALO + r0 - DIL * w, R), :]
                    acc = p if acc is None else acc + p
                    if chain and HQ == 2 and j == NB // 2 - 1:
                        att[T_, w, pinned(HALO + r0, R), :] = acc
                if chain and w % GQ == GQ - 1 and w < W - 1:
                    att[T_, w, pinned(HALO + r0, R), :] = acc
                    acc = None
                t.append(acc)
            t = [att[T_, w, here, :] if a is None else a for w, a in enumerate(t)]
            lane = jax.lax.broadcasted_iota(jnp.int32, (R, 128), 1)
            even = (lane & 1) == 0
            low16 = (lane & 16) == 0
            lg = []
            for w in range(W):
                a = t[w]
                a = a + jnp.where(even, pltpu.roll(a, 127, 1), pltpu.roll(a, 1, 1))
                a = a + jnp.where(low16, pltpu.roll(a, 112, 1), pltpu.roll(a, 16, 1))
                a = a * (DH ** -0.5 * LOG2E)
                if not chain or r0 < DIL * w:
                    row = jax.lax.broadcasted_iota(jnp.int32, (R, 128), 0)
                    a = jnp.where(pos0 + r0 + row - DIL * w >= 0, a, -1e9 * LOG2E)
                lg.append(a)
            mx = functools.reduce(jnp.maximum, lg)
            e = [jnp.exp2(a - mx) for a in lg]
            inv = 1.0 / functools.reduce(lambda a, b: a + b, e)
            return [a * inv for a in e]

        def mix(r0, pr, chain, R=R):
            here = pl.ds(HALO + r0, R)
            for j in range(NB):
                acc = None
                for w in range(W):
                    p = pr[w] * att[V_, j, pl.ds(HALO + r0 - DIL * w, R), :]
                    acc = p if acc is None else acc + p
                    if chain and HV == 2 and w == W // 2 - 1:
                        att[T_, j, pinned(HALO + r0, R), :] = acc
                att[O_, j, pinned(r0 // 2, R // 2), :] = pltpu.bitcast(acc.astype(bf16), f32)

        def out_proj(b, keep):
            x1 = xs[rows(b), :] + _dot(normed(O_), _cols(wo, 0, NB))
            xs[rows(b), :] = x1
            if keep:
                stage(Q_, x1)

        def gate_up(c0, fc):
            x2 = normed(X2_)
            g = _dot(x2, _cols(w1, c0, fc))
            u = _dot(x2, _cols(w3, c0, fc))
            h = (g * jax.nn.sigmoid(g) * u).astype(bf16)
            for c in range(fc):
                hb[c0 + c] = pltpu.bitcast(h[:, c * 128:(c + 1) * 128], f32)

        def hidden(c0, nc):
            return jnp.concatenate([pltpu.bitcast(hb[c0 + c], bf16) for c in range(nc)], axis=1)

        def load_x(lo, hi):
            def body(i, _):
                rs = pl.ds(pl.multiple_of(i * 64, 64), 64)
                xs[rs, :] = xb[rs, :].astype(f32)
                return 0
            jax.lax.fori_loop(lo // 64, hi // 64, body, 0)

        blk = n % NBLK
        prev = jnp.maximum(n - 1, 0) % NBLK
        nxt = (n + 1) % NBLK

        @pl.when(n == 0)
        def _start():
            start(cp_x0 + sum(cp_q, []))
            wait(cp_x0)
            load_x(0, RB)
            ln_loop(X1_, 0)
            start(sum(cp_kv[0] + cp_kv[1], []))

            def body(r, _):
                wait_one(cp_q, r)
                permute_rows(wq, r * PR, PR)
                return 0
            jax.lax.fori_loop(0, D // PR, body, 0)
            for i in range(3):
                start((cp_x1 + cp_wo, cp_gu[0], cp_gu[1])[i])

                def body(c, _, i=i):
                    if i < 2:
                        wait_one(cp_kv[i], c)
                    proj(i, True, c * (NB // CH), NB // CH)
                    if i < 2:
                        permute_rows(wqkv[i + 1], c * (D // CH), D // CH)
                    return 0
                jax.lax.fori_loop(0, CH, body, 0)
            wait(cp_x1)
            load_x(RB, 2 * RB)

            wait(cp_wo)
            permute_wo()

            def body(i, _):
                r0 = pl.multiple_of(i * R0, R0)
                mix(r0, probs(r0, 0, False, R0), False, R0)
                return 0
            jax.lax.fori_loop(0, RB // R0, body, 0)
            start(cp_x2 + cp_w2 + cp_xr)
            out_proj(0, False)
            if LM:
                for r0 in range(0, RB, 64):
                    ln_store(X1_, r0, xs[RB + r0:RB + r0 + 64, :])
            ln_loop(X2_, 0)
            if not LM:
                ln_loop(X1_, 1)

        @pl.when(n > 0)
        def _gate_up():
            def body(c, _):
                pl.when(n == 1)(lambda: wait_one(cp_gu, c))
                gate_up(c * FC, FC)
                return 0
            jax.lax.fori_loop(0, NG, body, 0)

        @pl.when(n == 1)
        def _wait_b():
            wait(cp_x2)
            load_x(2 * RB, 3 * RB)
            wait(cp_w2)

        @pl.when(n == 2)
        def _wait_x():
            wait(cp_xr)
            load_x(3 * RB, S)

        @pl.when(jnp.logical_and(n > 0, n < NJOB))
        def _attn():
            first = blk == 0
            stage(XN_, xs[rows(nxt), :])
            proj(Q_, first)
            proj(K_, first)
            proj(V_, first)
            pr = probs(0, blk * RB, True)
            for r0 in range(0, RB, R):
                if r0 % LR == 0:
                    x = staged(XN_, r0, LR)
                pr_next = probs(r0 + R, blk * RB, True) if r0 + R < RB and SP else None
                mix(r0, pr, True)
                if r0 % LR == 0:
                    ln_store(X1_, r0, x)
                pr = probs(r0 + R, blk * RB, True) if r0 + R < RB and not SP else pr_next
            xs[rows(prev), :] += _dot(hidden(0, DS), _cols(w2, 0, NB, slice(0, DS * 128)))
            out_proj(blk, True)
            x = staged(Q_, 0, L2)
            for r0 in range(0, RB, L2):
                x_next = staged(Q_, r0 + L2, L2) if r0 + L2 < RB else None
                ln_store(X2_, r0, x)
                x = x_next
            y = xs[rows(prev), :] + _dot(hidden(DS, FB - DS), _cols(w2, 0, NB, slice(DS * 128, F)))
            xs[rows(prev), :] = y
            o_ref[...] = y.astype(bf16)

        @pl.when(n == NJOB)
        def _last():
            def body(c, _):
                cs = pl.ds(pl.multiple_of(c * KC * 128, KC * 128), KC * 128)
                xs[rows(prev), :] += _dot(hidden(c * KC, KC), _cols(w2, 0, NB, cs))
                return 0
            jax.lax.fori_loop(0, FB // KC, body, 0)
            o_ref[...] = xs[rows(prev), :].astype(bf16)

    @jax.jit
    def run(A_x, A_wqkv, A_wo, B_x, B_w1, B_w3, B_w2):
        x = A_x.reshape(S, D)
        any_spec = pl.BlockSpec(memory_space=pl.ANY)
        out = pl.pallas_call(
            kernel,
            grid=(NJOB + 1,),
            in_specs=[any_spec] * 6,
            out_specs=pl.BlockSpec((RB, D), lambda i: (jnp.maximum(i - ((NL - 1) * NBLK + 1), 0), 0)),
            out_shape=jax.ShapeDtypeStruct((S, D), bf16),
            scratch_shapes=[
                *[pltpu.VMEM((NB, D, 128), bf16)] * 4,
                pltpu.VMEM((FB, D, 128), bf16), pltpu.VMEM((FB, D, 128), bf16), pltpu.VMEM((NB, F, 128), bf16),
                pltpu.VMEM((S, D), bf16), pltpu.VMEM((S, D), f32),
                pltpu.VMEM((8, NB, HALO + RB, 128), f32),
                pltpu.VMEM((FB, RB // 2, 128), f32),
                pltpu.SemaphoreType.DMA((8 + NG + D // PR + 2 * CH,)),
            ],
            compiler_params=pltpu.CompilerParams(
                dimension_semantics=("arbitrary",), vmem_limit_bytes=100 * 1024 * 1024, flags=flags),
        )(x, A_wqkv, A_wo, B_w1, B_w3, B_w2)
        return out.reshape(1, S, D)
    return run


_run = make()


def pallas_interleave_layers__sliding_local_dilated__glu_gated_swiglu__prompt_kernel(A_x, A_wqkv, A_wo, B_x, B_w1, B_w3, B_w2):
    return _run(A_x, A_wqkv, A_wo, B_x, B_w1, B_w3, B_w2)
```

```python
import functools

import jax
import jax.numpy as jnp
import jax.experimental.pallas as pl
import jax.experimental.pallas.tpu as pltpu

S, D, F = 2048, 1024, 3584
DH, W, DIL = 32, 8, 2
LAYERS = 2
RB = 256
NBLK = S // RB
NJOB = LAYERS * NBLK
HALO = 16
NB = D // 128
FB = F // 128
NG = 2
FC = FB // NG
DS = 25
AR = 16
QS = 256
KS = D // 2
LOG2E = 1.4426950408889634
Q_, K_, V_, T_, XA_, XF_, O_ = range(7)
f32, bf16 = jnp.float32, jnp.bfloat16


def _ln(x):
    d = x - jnp.mean(x, axis=-1, keepdims=True)
    v = jnp.mean(d * d, axis=-1, keepdims=True)
    return d * jax.lax.rsqrt(v + 1e-5)


def _dot(a, b):
    return jnp.dot(a, b, preferred_element_type=f32)


def _total(terms):
    return functools.reduce(jnp.add, terms)


def _cols(ref, start, count, rows=slice(None)):
    return jnp.concatenate([ref[start + c, rows, :] for c in range(count)], axis=1)


def _block(x, j):
    return x[:, j * 128:(j + 1) * 128]


def _swap_blocks(blocks, axis, unit):
    blocks = list(blocks)
    size = blocks[0].shape[axis]
    pos = jax.lax.broadcasted_iota(jnp.int32, blocks[0].shape, axis)
    for b in range(3):
        dist = unit << b
        low = (pos & dist) == 0
        for c in range(NB):
            if c & (1 << b):
                continue
            lo, hi = blocks[c], blocks[c | (1 << b)]
            blocks[c] = jnp.where(low, lo, pltpu.roll(hi, dist, axis))
            blocks[c | (1 << b)] = jnp.where(low, pltpu.roll(lo, size - dist, axis), hi)
    return blocks


def _kernel(x_hbm, wqkv_hbm, wo_hbm, w1_hbm, w3_hbm, w2_hbm, o_ref,
            wq, wk, wv, wo, w1, w3, w2, xb, xs, att, hb, sems):
    n = pl.program_id(0)
    blk = n % NBLK
    prev = jnp.maximum(n - 1, 0) % NBLK
    wqkv = (wq, wk, wv)
    zero = (n // 4096) * 8

    def rows(b):
        if isinstance(b, int):
            return slice(b * RB, (b + 1) * RB)
        return pl.ds(pl.multiple_of(b * RB, RB), RB)

    def pinned(r0, size):
        return pl.ds(pl.multiple_of(r0 + zero, 8), size)

    def row_copy(lo, hi, sem):
        return [pltpu.make_async_copy(x_hbm.at[pl.ds(lo, hi - lo)], xb.at[pl.ds(lo, hi - lo)], sems.at[sem])]

    def col_copies(src, dst, lo, hi, sem):
        return [pltpu.make_async_copy(src.at[:, pl.ds(c * 128, 128)], dst.at[c], sems.at[sem])
                for c in range(lo, hi)]

    def slab_copies(i, size, sem):
        return [[pltpu.make_async_copy(wqkv_hbm.at[pl.ds(r * size, size), pl.ds(i * D + c * 128, 128)],
                                       wqkv[i].at[c, pl.ds(r * size, size)], sems.at[sem + r])
                 for c in range(NB)] for r in range(D // size)]

    cp_x0, cp_x1, cp_xr = row_copy(0, RB, 0), row_copy(RB, 2 * RB, 1), row_copy(2 * RB, S, 2)
    cp_wo = col_copies(wo_hbm, wo, 0, NB, 3)
    cp_w2 = col_copies(w2_hbm, w2, 0, NB, 4)
    cp_gu = [col_copies(w1_hbm, w1, g * FC, (g + 1) * FC, 5 + g) + col_copies(w3_hbm, w3, g * FC, (g + 1) * FC, 5 + g)
             for g in range(NG)]
    cp_q = slab_copies(Q_, QS, 5 + NG)
    cp_kv = [slab_copies(i, KS, 5 + NG + D // QS + (i - K_) * (D // KS)) for i in (K_, V_)]

    def start(cps):
        for c in cps:
            c.start()

    def wait(cps):
        for c in cps:
            c.wait()

    def wait_one(groups, k):
        for i, cps in enumerate(groups):
            pl.when(k == i)(functools.partial(wait, cps))

    def permute_cols(w, r0, size):
        rs = pl.ds(pl.multiple_of(r0, size), size)
        blocks = _swap_blocks([pltpu.bitcast(w[c, rs, :], jnp.uint32) for c in range(NB)], 1, 2)
        for c in range(NB):
            w[c, rs, :] = pltpu.bitcast(blocks[c], bf16)

    def permute_wo_rows():
        def body(m, _):
            rs = [pl.ds(pl.multiple_of(c * 128 + m * 16, 16), 16) for c in range(NB)]
            blocks = _swap_blocks([pltpu.bitcast(_cols(wo, 0, NB, r), jnp.uint32) for r in rs], 0, 1)
            for r, words in zip(rs, blocks):
                y = pltpu.bitcast(words, bf16)
                for j in range(NB):
                    wo[j, r, :] = _block(y, j)
            return 0
        jax.lax.fori_loop(0, 128 // 16, body, 0)

    def packed(plane):
        return jnp.concatenate([pltpu.bitcast(att[plane, j, 0:RB // 2, :], bf16) for j in range(NB)], axis=1)

    def hidden(c0, count):
        return jnp.concatenate([pltpu.bitcast(hb[c0 + c], bf16) for c in range(count)], axis=1)

    def ln_store(plane, r0, x):
        y = pltpu.bitcast(_ln(x).astype(bf16), f32)
        dst = pinned(r0 // 2, x.shape[0] // 2)
        for j in range(NB):
            att[plane, j, dst, :] = _block(y, j)

    def ln_first_block(plane):
        def body(i, _):
            r0 = pl.multiple_of(i * 128, 128)
            ln_store(plane, r0, xs[pl.ds(r0, 128), :])
            return 0
        jax.lax.fori_loop(0, RB // 128, body, 0)

    def load_x(lo, hi):
        def body(i, _):
            rs = pl.ds(pl.multiple_of(i * 64, 64), 64)
            xs[rs, :] = xb[rs, :].astype(f32)
            return 0
        jax.lax.fori_loop(lo // 64, hi // 64, body, 0)

    def project(i, first, j0=0, count=NB):
        y = _dot(packed(XA_), _cols(wqkv[i], j0, count))
        for j in range(count):
            yj = _block(y, j)
            if i != Q_:
                halo = jnp.broadcast_to(yj[0:1, :], (HALO, 128))
                if first is not True:
                    halo = jnp.where(first, halo, att[i, j0 + j, RB:RB + HALO, :])
                att[i, j0 + j, 0:HALO, :] = halo
            att[i, j0 + j, HALO:HALO + RB, :] = yj

    def attend(r0, size, pos0):
        static = isinstance(r0, int)
        here = pl.ds(HALO + r0, size)
        q = [att[Q_, j, here, :] for j in range(NB)]
        for w in range(W):
            part = _total(q[j] * att[K_, j, pl.ds(HALO + r0 - DIL * w, size), :] for j in range(NB))
            if w < W - 1:
                att[T_, w, pinned(HALO + r0, size), :] = part
        parts = [att[T_, w, here, :] for w in range(W - 1)] + [part]
        lane = jax.lax.broadcasted_iota(jnp.int32, (size, 128), 1)
        row = jax.lax.broadcasted_iota(jnp.int32, (size, 128), 0)
        even, low = (lane & 1) == 0, (lane & 16) == 0
        logits = []
        for w, a in enumerate(parts):
            a = a + jnp.where(even, pltpu.roll(a, 127, 1), pltpu.roll(a, 1, 1))
            a = a + jnp.where(low, pltpu.roll(a, 112, 1), pltpu.roll(a, 16, 1))
            a = a * (DH ** -0.5 * LOG2E)
            if not static or r0 < DIL * w:
                a = jnp.where(pos0 + r0 + row - DIL * w >= 0, a, -1e9 * LOG2E)
            logits.append(a)
        top = functools.reduce(jnp.maximum, logits)
        e = [jnp.exp2(a - top) for a in logits]
        inv = 1.0 / _total(e)
        for j in range(NB):
            acc = _total(e[w] * att[V_, j, pl.ds(HALO + r0 - DIL * w, size), :] for w in range(W))
            att[O_, j, pinned(r0 // 2, size // 2), :] = pltpu.bitcast((acc * inv).astype(bf16), f32)

    def out_proj(b):
        y = xs[rows(b), :] + _dot(packed(O_), _cols(wo, 0, NB))
        xs[rows(b), :] = y
        return y

    @pl.when(n == 0)
    def _start():
        start(cp_x0 + sum(cp_q, []))
        wait(cp_x0)
        load_x(0, RB)
        ln_first_block(XA_)
        start(sum(cp_kv[0] + cp_kv[1], []))

        def permute_q(r, _):
            wait_one(cp_q, r)
            permute_cols(wq, r * QS, QS)
            return 0
        jax.lax.fori_loop(0, D // QS, permute_q, 0)

        for i in (Q_, K_, V_):
            start((cp_x1 + cp_wo, cp_gu[0], cp_gu[1])[i])

            def half(c, _, i=i):
                if i != V_:
                    wait_one(cp_kv[i], c)
                project(i, True, c * (NB * KS // D), NB * KS // D)
                if i != V_:
                    permute_cols(wqkv[i + 1], c * KS, KS)
                return 0
            jax.lax.fori_loop(0, D // KS, half, 0)

        wait(cp_x1)
        load_x(RB, 2 * RB)
        wait(cp_wo)
        permute_wo_rows()

        def attend_rows(i, _):
            attend(pl.multiple_of(i * 128, 128), 128, 0)
            return 0
        jax.lax.fori_loop(0, RB // 128, attend_rows, 0)
        start(cp_w2 + cp_xr)
        out_proj(0)
        ln_first_block(XF_)

    @pl.when(n == 2)
    def _rest_of_x():
        wait(cp_xr)
        load_x(2 * RB, S)

    @pl.when(n > 0)
    def _gate_up():
        def body(g, _):
            pl.when(n == 1)(lambda: wait_one(cp_gu, g))
            gate = _dot(packed(XF_), _cols(w1, g * FC, FC))
            for r in range(0, RB // NG, 16):
                r0 = pl.multiple_of(g * (RB // NG) + r, 16)
                ln_store(XA_, r0, xs[pl.ds(pl.multiple_of(blk * RB + r0, 16), 16), :])
            up = _dot(packed(XF_), _cols(w3, g * FC, FC))
            h = (gate * jax.nn.sigmoid(gate) * up).astype(bf16)
            for c in range(FC):
                hb[g * FC + c] = pltpu.bitcast(_block(h, c), f32)
            return 0
        jax.lax.fori_loop(0, NG, body, 0)

    @pl.when(n == 1)
    def _wait_w2():
        wait(cp_w2)

    @pl.when(jnp.logical_and(n > 0, n < NJOB))
    def _main():
        for i in (Q_, K_, V_):
            project(i, blk == 0)
        for r0 in range(0, RB, AR):
            attend(r0, AR, blk * RB)
        xs[rows(prev), :] += _dot(hidden(0, DS), _cols(w2, 0, NB, slice(0, DS * 128)))

        x1 = out_proj(blk)
        for j in range(NB):
            att[Q_, j, HALO:HALO + RB, :] = _block(x1, j)

        def x1_rows(r0):
            return jnp.concatenate([att[Q_, j, HALO + r0:HALO + r0 + 32, :] for j in range(NB)], axis=1)

        cur = x1_rows(0)
        for r0 in range(0, RB, 32):
            nxt = x1_rows(r0 + 32) if r0 + 32 < RB else None
            ln_store(XF_, r0, cur)
            cur = nxt

        y = xs[rows(prev), :] + _dot(hidden(DS, FB - DS), _cols(w2, 0, NB, slice(DS * 128, F)))
        xs[rows(prev), :] = y
        o_ref[...] = y.astype(bf16)

    @pl.when(n == NJOB)
    def _last():
        def body(c, _):
            ks = pl.ds(pl.multiple_of(c * 512, 512), 512)
            xs[rows(prev), :] += _dot(hidden(c * 4, 4), _cols(w2, 0, NB, ks))
            return 0
        jax.lax.fori_loop(0, F // 512, body, 0)
        o_ref[...] = xs[rows(prev), :].astype(bf16)


@jax.jit
def pallas_interleave_layers__sliding_local_dilated__glu_gated_swiglu__prompt_kernel(
    A_x: jax.Array,
    A_wqkv: jax.Array,
    A_wo: jax.Array,
    B_x: jax.Array,
    B_w1: jax.Array,
    B_w3: jax.Array,
    B_w2: jax.Array,
):
    del B_x
    first_out = (LAYERS - 1) * NBLK + 1
    out = pl.pallas_call(
        _kernel,
        grid=(NJOB + 1,),
        in_specs=[pl.BlockSpec(memory_space=pl.ANY)] * 6,
        out_specs=pl.BlockSpec((RB, D), lambda i: (jnp.maximum(i - first_out, 0), 0)),
        out_shape=jax.ShapeDtypeStruct((S, D), bf16),
        scratch_shapes=[
            *[pltpu.VMEM((NB, D, 128), bf16)] * 4,
            *[pltpu.VMEM((FB, D, 128), bf16)] * 2,
            pltpu.VMEM((NB, F, 128), bf16),
            pltpu.VMEM((S, D), bf16),
            pltpu.VMEM((S, D), f32),
            pltpu.VMEM((7, NB, HALO + RB, 128), f32),
            pltpu.VMEM((FB, RB // 2, 128), f32),
            pltpu.SemaphoreType.DMA((5 + NG + D // QS + 2 * (D // KS),)),
        ],
        compiler_params=pltpu.CompilerParams(
            dimension_semantics=("arbitrary",), vmem_limit_bytes=100 * 1024 * 1024),
    )(A_x.reshape(S, D), A_wqkv, A_wo, B_w1, B_w3, B_w2)
    return out.reshape(1, S, D)
```

```python
import functools

import jax
import jax.numpy as jnp
import jax.experimental.pallas as pl
import jax.experimental.pallas.tpu as pltpu

S, D, F = 2048, 1024, 3584
DH, W, DIL = 32, 8, 2
LAYERS = 2
RB = 256
NBLK = S // RB
NJOB = LAYERS * NBLK
HALO = 16
NB = D // 128
FB = F // 128
NG = 2
FC = FB // NG
DS = 25
AR = 16
QS = 256
KS = D // 2
LOG2E = 1.4426950408889634
Q_, K_, V_, T_, XA_, XF_, O_ = range(7)
f32, bf16 = jnp.float32, jnp.bfloat16


def _ln(x):
    d = x - jnp.mean(x, axis=-1, keepdims=True)
    v = jnp.mean(d * d, axis=-1, keepdims=True)
    return d * jax.lax.rsqrt(v + 1e-5)


def _dot(a, b):
    return jnp.dot(a, b, preferred_element_type=f32)


def _total(terms):
    return functools.reduce(jnp.add, terms)


def _cols(ref, start, count, rows=slice(None)):
    return jnp.concatenate([ref[start + c, rows, :] for c in range(count)], axis=1)


def _block(x, j):
    return x[:, j * 128:(j + 1) * 128]


def _swap_blocks(blocks, axis, unit):
    blocks = list(blocks)
    size = blocks[0].shape[axis]
    pos = jax.lax.broadcasted_iota(jnp.int32, blocks[0].shape, axis)
    for b in range(3):
        dist = unit << b
        low = (pos & dist) == 0
        for c in range(NB):
            if c & (1 << b):
                continue
            lo, hi = blocks[c], blocks[c | (1 << b)]
            blocks[c] = jnp.where(low, lo, pltpu.roll(hi, dist, axis))
            blocks[c | (1 << b)] = jnp.where(low, pltpu.roll(lo, size - dist, axis), hi)
    return blocks


def _kernel(x_hbm, wqkv_hbm, wo_hbm, w1_hbm, w3_hbm, w2_hbm, o_ref,
            wq, wk, wv, wo, w1, w3, w2, xb, xs, att, hb, sems):
    n = pl.program_id(0)
    blk = n % NBLK
    prev = jnp.maximum(n - 1, 0) % NBLK
    wqkv = (wq, wk, wv)
    zero = (n // 4096) * 8

    def rows(b):
        if isinstance(b, int):
            return slice(b * RB, (b + 1) * RB)
        return pl.ds(pl.multiple_of(b * RB, RB), RB)

    def pinned(r0, size):
        return pl.ds(pl.multiple_of(r0 + zero, 8), size)

    def row_copy(lo, hi, sem):
        return [pltpu.make_async_copy(x_hbm.at[pl.ds(lo, hi - lo)], xb.at[pl.ds(lo, hi - lo)], sems.at[sem])]

    def col_copies(src, dst, lo, hi, sem):
        return [pltpu.make_async_copy(src.at[:, pl.ds(c * 128, 128)], dst.at[c], sems.at[sem])
                for c in range(lo, hi)]

    def slab_copies(i, size, sem):
        return [[pltpu.make_async_copy(wqkv_hbm.at[pl.ds(r * size, size), pl.ds(i * D + c * 128, 128)],
                                       wqkv[i].at[c, pl.ds(r * size, size)], sems.at[sem + r])
                 for c in range(NB)] for r in range(D // size)]

    cp_x0, cp_x1, cp_xr = row_copy(0, RB, 0), row_copy(RB, 2 * RB, 1), row_copy(2 * RB, S, 2)
    cp_wo = col_copies(wo_hbm, wo, 0, NB, 3)
    cp_w2 = col_copies(w2_hbm, w2, 0, NB, 4)
    cp_gu = [col_copies(w1_hbm, w1, g * FC, (g + 1) * FC, 5 + g) + col_copies(w3_hbm, w3, g * FC, (g + 1) * FC, 5 + g)
             for g in range(NG)]
    cp_q = slab_copies(Q_, QS, 5 + NG)
    cp_kv = [slab_copies(i, KS, 5 + NG + D // QS + (i - K_) * (D // KS)) for i in (K_, V_)]

    def start(cps):
        for c in cps:
            c.start()

    def wait(cps):
        for c in cps:
            c.wait()

    def wait_one(groups, k):
        for i, cps in enumerate(groups):
            pl.when(k == i)(functools.partial(wait, cps))

    def permute_cols(w, r0, size):
        rs = pl.ds(pl.multiple_of(r0, size), size)
        blocks = _swap_blocks([pltpu.bitcast(w[c, rs, :], jnp.uint32) for c in range(NB)], 1, 2)
        for c in range(NB):
            w[c, rs, :] = pltpu.bitcast(blocks[c], bf16)

    def permute_wo_rows():
        def body(m, _):
            rs = [pl.ds(pl.multiple_of(c * 128 + m * 16, 16), 16) for c in range(NB)]
            blocks = _swap_blocks([pltpu.bitcast(_cols(wo, 0, NB, r), jnp.uint32) for r in rs], 0, 1)
            for r, words in zip(rs, blocks):
                y = pltpu.bitcast(words, bf16)
                for j in range(NB):
                    wo[j, r, :] = _block(y, j)
            return 0
        jax.lax.fori_loop(0, 128 // 16, body, 0)

    def packed(plane):
        return jnp.concatenate([pltpu.bitcast(att[plane, j, 0:RB // 2, :], bf16) for j in range(NB)], axis=1)

    def hidden(c0, count):
        return jnp.concatenate([pltpu.bitcast(hb[c0 + c], bf16) for c in range(count)], axis=1)

    def ln_store(plane, r0, x):
        y = pltpu.bitcast(_ln(x).astype(bf16), f32)
        dst = pinned(r0 // 2, x.shape[0] // 2)
        for j in range(NB):
            att[plane, j, dst, :] = _block(y, j)

    def ln_first_block(plane):
        def body(i, _):
            r0 = pl.multiple_of(i * 128, 128)
            ln_store(plane, r0, xs[pl.ds(r0, 128), :])
            return 0
        jax.lax.fori_loop(0, RB // 128, body, 0)

    def load_x(lo, hi):
        def body(i, _):
            rs = pl.ds(pl.multiple_of(i * 64, 64), 64)
            xs[rs, :] = xb[rs, :].astype(f32)
            return 0
        jax.lax.fori_loop(lo // 64, hi // 64, body, 0)

    def project(i, first, j0=0, count=NB):
        y = _dot(packed(XA_), _cols(wqkv[i], j0, count))
        for j in range(count):
            yj = _block(y, j)
            if i != Q_:
                halo = jnp.broadcast_to(yj[0:1, :], (HALO, 128))
                if first is not True:
                    halo = jnp.where(first, halo, att[i, j0 + j, RB:RB + HALO, :])
                att[i, j0 + j, 0:HALO, :] = halo
            att[i, j0 + j, HALO:HALO + RB, :] = yj

    def attend(r0, size, pos0):
        static = isinstance(r0, int)
        here = pl.ds(HALO + r0, size)
        q = [att[Q_, j, here, :] for j in range(NB)]
        for w in range(W):
            part = _total(q[j] * att[K_, j, pl.ds(HALO + r0 - DIL * w, size), :] for j in range(NB))
            if w < W - 1:
                att[T_, w, pinned(HALO + r0, size), :] = part
        parts = [att[T_, w, here, :] for w in range(W - 1)] + [part]
        lane = jax.lax.broadcasted_iota(jnp.int32, (size, 128), 1)
        row = jax.lax.broadcasted_iota(jnp.int32, (size, 128), 0)
        even, low = (lane & 1) == 0, (lane & 16) == 0
        logits = []
        for w, a in enumerate(parts):
            a = a + jnp.where(even, pltpu.roll(a, 127, 1), pltpu.roll(a, 1, 1))
            a = a + jnp.where(low, pltpu.roll(a, 112, 1), pltpu.roll(a, 16, 1))
            a = a * (DH ** -0.5 * LOG2E)
            if not static or r0 < DIL * w:
                a = jnp.where(pos0 + r0 + row - DIL * w >= 0, a, -1e9 * LOG2E)
            logits.append(a)
        top = functools.reduce(jnp.maximum, logits)
        e = [jnp.exp2(a - top) for a in logits]
        inv = 1.0 / _total(e)
        for j in range(NB):
            acc = _total(e[w] * att[V_, j, pl.ds(HALO + r0 - DIL * w, size), :] for w in range(W))
            att[O_, j, pinned(r0 // 2, size // 2), :] = pltpu.bitcast((acc * inv).astype(bf16), f32)

    def out_proj(b):
        y = xs[rows(b), :] + _dot(packed(O_), _cols(wo, 0, NB))
        xs[rows(b), :] = y
        return y

    @pl.when(n == 0)
    def _start():
        start(cp_x0 + sum(cp_q, []))
        wait(cp_x0)
        load_x(0, RB)
        ln_first_block(XA_)
        start(sum(cp_kv[0] + cp_kv[1], []))

        def permute_q(r, _):
            wait_one(cp_q, r)
            permute_cols(wq, r * QS, QS)
            return 0
        jax.lax.fori_loop(0, D // QS, permute_q, 0)

        for i in (Q_, K_, V_):
            start((cp_x1 + cp_wo, cp_gu[0], cp_gu[1])[i])

            def half(c, _, i=i):
                if i != V_:
                    wait_one(cp_kv[i], c)
                project(i, True, c * (NB * KS // D), NB * KS // D)
                if i != V_:
                    permute_cols(wqkv[i + 1], c * KS, KS)
                return 0
            jax.lax.fori_loop(0, D // KS, half, 0)

        wait(cp_x1)
        load_x(RB, 2 * RB)
        wait(cp_wo)
        permute_wo_rows()

        def attend_rows(i, _):
            attend(pl.multiple_of(i * 128, 128), 128, 0)
            return 0
        jax.lax.fori_loop(0, RB // 128, attend_rows, 0)
        start(cp_w2 + cp_xr)
        out_proj(0)
        ln_first_block(XF_)

    @pl.when(n == 2)
    def _rest_of_x():
        wait(cp_xr)
        load_x(2 * RB, S)

    @pl.when(n > 0)
    def _gate_up():
        def body(g, _):
            pl.when(n == 1)(lambda: wait_one(cp_gu, g))
            gate = _dot(packed(XF_), _cols(w1, g * FC, FC))
            for r in range(0, RB // NG, 16):
                r0 = pl.multiple_of(g * (RB // NG) + r, 16)
                ln_store(XA_, r0, xs[pl.ds(pl.multiple_of(blk * RB + r0, 16), 16), :])
            up = _dot(packed(XF_), _cols(w3, g * FC, FC))
            half = 0.5 * gate
            h = ((half * jnp.tanh(half) + half) * up).astype(bf16)
            for c in range(FC):
                hb[g * FC + c] = pltpu.bitcast(_block(h, c), f32)
            return 0
        jax.lax.fori_loop(0, NG, body, 0)

    @pl.when(n == 1)
    def _wait_w2():
        wait(cp_w2)

    @pl.when(jnp.logical_and(n > 0, n < NJOB))
    def _main():
        for i in (Q_, K_, V_):
            project(i, blk == 0)
        for r0 in range(0, RB, AR):
            attend(r0, AR, blk * RB)
        xs[rows(prev), :] += _dot(hidden(0, DS), _cols(w2, 0, NB, slice(0, DS * 128)))

        x1 = out_proj(blk)
        for j in range(NB):
            att[Q_, j, HALO:HALO + RB, :] = _block(x1, j)

        def x1_rows(r0):
            return jnp.concatenate([att[Q_, j, HALO + r0:HALO + r0 + 32, :] for j in range(NB)], axis=1)

        cur = x1_rows(0)
        for r0 in range(0, RB, 32):
            nxt = x1_rows(r0 + 32) if r0 + 32 < RB else None
            ln_store(XF_, r0, cur)
            cur = nxt

        y = xs[rows(prev), :] + _dot(hidden(DS, FB - DS), _cols(w2, 0, NB, slice(DS * 128, F)))
        xs[rows(prev), :] = y
        o_ref[...] = y.astype(bf16)

    @pl.when(n == NJOB)
    def _last():
        def body(c, _):
            ks = pl.ds(pl.multiple_of(c * 896, 128), 896)
            xs[rows(prev), :] += _dot(hidden(c * 7, 7), _cols(w2, 0, NB, ks))
            return 0
        jax.lax.fori_loop(0, F // 896, body, 0)
        o_ref[...] = xs[rows(prev), :].astype(bf16)


@jax.jit
def pallas_interleave_layers__sliding_local_dilated__glu_gated_swiglu__prompt_kernel(
    A_x: jax.Array,
    A_wqkv: jax.Array,
    A_wo: jax.Array,
    B_x: jax.Array,
    B_w1: jax.Array,
    B_w3: jax.Array,
    B_w2: jax.Array,
):
    del B_x
    first_out = (LAYERS - 1) * NBLK + 1
    out = pl.pallas_call(
        _kernel,
        grid=(NJOB + 1,),
        in_specs=[pl.BlockSpec(memory_space=pl.ANY)] * 6,
        out_specs=pl.BlockSpec((RB, D), lambda i: (jnp.maximum(i - first_out, 0), 0)),
        out_shape=jax.ShapeDtypeStruct((S, D), bf16),
        scratch_shapes=[
            *[pltpu.VMEM((NB, D, 128), bf16)] * 4,
            *[pltpu.VMEM((FB, D, 128), bf16)] * 2,
            pltpu.VMEM((NB, F, 128), bf16),
            pltpu.VMEM((S, D), bf16),
            pltpu.VMEM((S, D), f32),
            pltpu.VMEM((7, NB, HALO + RB, 128), f32),
            pltpu.VMEM((FB, RB // 2, 128), f32),
            pltpu.SemaphoreType.DMA((5 + NG + D // QS + 2 * (D // KS),)),
        ],
        compiler_params=pltpu.CompilerParams(
            dimension_semantics=("arbitrary",), vmem_limit_bytes=100 * 1024 * 1024),
    )(A_x.reshape(S, D), A_wqkv, A_wo, B_w1, B_w3, B_w2)
    return out.reshape(1, S, D)
```

```python
import functools

import jax
import jax.numpy as jnp
import jax.experimental.pallas as pl
import jax.experimental.pallas.tpu as pltpu

S, D, F = 2048, 1024, 3584
DH, W, DIL = 32, 8, 2
LAYERS = 2
RB = 256
NBLK = S // RB
NJOB = LAYERS * NBLK
HALO = 16
NB = D // 128
FB = F // 128
NG = 2
FC = FB // NG
DS = 24
AR = 16
QS = 256
KS = D // 2
LOG2E = 1.4426950408889634
Q_, K_, V_, T_, XA_, XF_, O_ = range(7)
f32, bf16 = jnp.float32, jnp.bfloat16


def _ln(x):
    d = x - jnp.mean(x, axis=-1, keepdims=True)
    v = jnp.mean(d * d, axis=-1, keepdims=True)
    return d * jax.lax.rsqrt(v + 1e-5)


def _dot(a, b):
    return jnp.dot(a, b, preferred_element_type=f32)


def _total(terms):
    return functools.reduce(jnp.add, terms)


def _cols(ref, start, count, rows=slice(None)):
    return jnp.concatenate([ref[start + c, rows, :] for c in range(count)], axis=1)


def _block(x, j):
    return x[:, j * 128:(j + 1) * 128]


def _swap_blocks(blocks, axis, unit):
    blocks = list(blocks)
    size = blocks[0].shape[axis]
    pos = jax.lax.broadcasted_iota(jnp.int32, blocks[0].shape, axis)
    for b in range(3):
        dist = unit << b
        low = (pos & dist) == 0
        for c in range(NB):
            if c & (1 << b):
                continue
            lo, hi = blocks[c], blocks[c | (1 << b)]
            blocks[c] = jnp.where(low, lo, pltpu.roll(hi, dist, axis))
            blocks[c | (1 << b)] = jnp.where(low, pltpu.roll(lo, size - dist, axis), hi)
    return blocks


def _kernel(x_hbm, wqkv_hbm, wo_hbm, w1_hbm, w3_hbm, w2_hbm, o_ref,
            wq, wk, wv, wo, w1, w3, w2, xb, xs, att, hb, sems):
    n = pl.program_id(0)
    blk = n % NBLK
    prev = jnp.maximum(n - 1, 0) % NBLK
    wqkv = (wq, wk, wv)
    zero = (n // 4096) * 8

    def rows(b):
        if isinstance(b, int):
            return slice(b * RB, (b + 1) * RB)
        return pl.ds(pl.multiple_of(b * RB, RB), RB)

    def pinned(r0, size):
        return pl.ds(pl.multiple_of(r0 + zero, 8), size)

    def row_copy(lo, hi, sem):
        return [pltpu.make_async_copy(x_hbm.at[pl.ds(lo, hi - lo)], xb.at[pl.ds(lo, hi - lo)], sems.at[sem])]

    def col_copies(src, dst, lo, hi, sem):
        return [pltpu.make_async_copy(src.at[:, pl.ds(c * 128, 128)], dst.at[c], sems.at[sem])
                for c in range(lo, hi)]

    def slab_copies(i, size, sem):
        return [[pltpu.make_async_copy(wqkv_hbm.at[pl.ds(r * size, size), pl.ds(i * D + c * 128, 128)],
                                       wqkv[i].at[c, pl.ds(r * size, size)], sems.at[sem + r])
                 for c in range(NB)] for r in range(D // size)]

    cp_x0, cp_x1, cp_xr = row_copy(0, RB, 0), row_copy(RB, 2 * RB, 1), row_copy(2 * RB, S, 2)
    cp_wo = col_copies(wo_hbm, wo, 0, NB, 3)
    cp_w2 = col_copies(w2_hbm, w2, 0, NB, 4)
    cp_gu = [col_copies(w1_hbm, w1, g * FC, (g + 1) * FC, 5 + g) + col_copies(w3_hbm, w3, g * FC, (g + 1) * FC, 5 + g)
             for g in range(NG)]
    cp_q = slab_copies(Q_, QS, 5 + NG)
    cp_kv = [slab_copies(i, KS, 5 + NG + D // QS + (i - K_) * (D // KS)) for i in (K_, V_)]

    def start(cps):
        for c in cps:
            c.start()

    def wait(cps):
        for c in cps:
            c.wait()

    def wait_one(groups, k):
        for i, cps in enumerate(groups):
            pl.when(k == i)(functools.partial(wait, cps))

    def permute_cols(w, r0, size):
        rs = pl.ds(pl.multiple_of(r0, size), size)
        blocks = _swap_blocks([pltpu.bitcast(w[c, rs, :], jnp.uint32) for c in range(NB)], 1, 2)
        for c in range(NB):
            w[c, rs, :] = pltpu.bitcast(blocks[c], bf16)

    def permute_wo_rows():
        def body(m, _):
            rs = [pl.ds(pl.multiple_of(c * 128 + m * 16, 16), 16) for c in range(NB)]
            blocks = _swap_blocks([pltpu.bitcast(_cols(wo, 0, NB, r), jnp.uint32) for r in rs], 0, 1)
            for r, words in zip(rs, blocks):
                y = pltpu.bitcast(words, bf16)
                for j in range(NB):
                    wo[j, r, :] = _block(y, j)
            return 0
        jax.lax.fori_loop(0, 128 // 16, body, 0)

    def packed(plane):
        return jnp.concatenate([pltpu.bitcast(att[plane, j, 0:RB // 2, :], bf16) for j in range(NB)], axis=1)

    def hidden(c0, count):
        return jnp.concatenate([pltpu.bitcast(hb[c0 + c], bf16) for c in range(count)], axis=1)

    def ln_store(plane, r0, x):
        y = pltpu.bitcast(_ln(x).astype(bf16), f32)
        dst = pinned(r0 // 2, x.shape[0] // 2)
        for j in range(NB):
            att[plane, j, dst, :] = _block(y, j)
        return y

    def ln_first_block(plane):
        def body(i, _):
            r0 = pl.multiple_of(i * 128, 128)
            ln_store(plane, r0, xs[pl.ds(r0, 128), :])
            return 0
        jax.lax.fori_loop(0, RB // 128, body, 0)

    def load_x(lo, hi):
        def body(i, _):
            rs = pl.ds(pl.multiple_of(i * 64, 64), 64)
            xs[rs, :] = xb[rs, :].astype(f32)
            return 0
        jax.lax.fori_loop(lo // 64, hi // 64, body, 0)

    def project(i, first, j0=0, count=NB):
        y = _dot(packed(XA_), _cols(wqkv[i], j0, count))
        for j in range(count):
            yj = _block(y, j)
            if i != Q_:
                halo = jnp.broadcast_to(yj[0:1, :], (HALO, 128))
                if first is not True:
                    halo = jnp.where(first, halo, att[i, j0 + j, RB:RB + HALO, :])
                att[i, j0 + j, 0:HALO, :] = halo
            att[i, j0 + j, HALO:HALO + RB, :] = yj

    def attend(r0, size, pos0):
        static = isinstance(r0, int)
        here = pl.ds(HALO + r0, size)
        q = [att[Q_, j, here, :] for j in range(NB)]
        parts = []
        for w in range(W):
            part = _total(q[j] * att[K_, j, pl.ds(HALO + r0 - DIL * w, size), :] for j in range(NB))
            if w < W - 1:
                att[T_, w, pinned(HALO + r0, 8), :] = part[size - 8:]
            parts.append(part)
        lane = jax.lax.broadcasted_iota(jnp.int32, (size, 128), 1)
        row = jax.lax.broadcasted_iota(jnp.int32, (size, 128), 0)
        even, low = (lane & 1) == 0, (lane & 16) == 0
        logits = []
        for w, a in enumerate(parts):
            a = a + jnp.where(even, pltpu.roll(a, 127, 1), pltpu.roll(a, 1, 1))
            a = a + jnp.where(low, pltpu.roll(a, 112, 1), pltpu.roll(a, 16, 1))
            a = a * (DH ** -0.5 * LOG2E)
            if not static or r0 < DIL * w:
                a = jnp.where(pos0 + r0 + row - DIL * w >= 0, a, -1e9 * LOG2E)
            logits.append(a)
        top = functools.reduce(jnp.maximum, logits)
        e = [jnp.exp2(a - top) for a in logits]
        inv = 1.0 / _total(e)
        for j in range(NB):
            acc = _total(e[w] * att[V_, j, pl.ds(HALO + r0 - DIL * w, size), :] for w in range(W))
            att[O_, j, pinned(r0 // 2, size // 2), :] = pltpu.bitcast((acc * inv).astype(bf16), f32)

    def out_proj(b):
        y = xs[rows(b), :] + _dot(packed(O_), _cols(wo, 0, NB))
        xs[rows(b), :] = y
        return y

    @pl.when(n == 0)
    def _start():
        start(cp_x0 + sum(cp_q, []))
        wait(cp_x0)
        load_x(0, RB)
        ln_first_block(XA_)
        start(sum(cp_kv[0] + cp_kv[1], []))

        def permute_q(r, _):
            wait_one(cp_q, r)
            permute_cols(wq, r * QS, QS)
            return 0
        jax.lax.fori_loop(0, D // QS, permute_q, 0)

        for i in (Q_, K_, V_):
            start((cp_x1 + cp_wo, cp_gu[0], cp_gu[1])[i])

            def half(c, _, i=i):
                if i != V_:
                    wait_one(cp_kv[i], c)
                project(i, True, c * (NB * KS // D), NB * KS // D)
                if i != V_:
                    permute_cols(wqkv[i + 1], c * KS, KS)
                return 0
            jax.lax.fori_loop(0, D // KS, half, 0)

        wait(cp_x1)
        load_x(RB, 2 * RB)
        wait(cp_wo)
        permute_wo_rows()

        def attend_rows(i, _):
            attend(pl.multiple_of(i * 128, 128), 128, 0)
            return 0
        jax.lax.fori_loop(0, RB // 128, attend_rows, 0)
        start(cp_w2 + cp_xr)
        out_proj(0)
        ln_first_block(XF_)

    @pl.when(n == 2)
    def _rest_of_x():
        wait(cp_xr)
        load_x(2 * RB, S)

    @pl.when(n > 0)
    def _gate_up():
        def body(g, _):
            pl.when(n == 1)(lambda: wait_one(cp_gu, g))
            gate = _dot(packed(XF_), _cols(w1, g * FC, FC))
            for r in range(0, RB // NG, 16):
                r0 = pl.multiple_of(g * (RB // NG) + r, 16)
                y = ln_store(XA_, r0, xs[pl.ds(pl.multiple_of(blk * RB + r0, 16), 16), :])
                xs[pinned(S, 8), 0:128] = y[0:8, 0:128]
            up = _dot(packed(XF_), _cols(w3, g * FC, FC))
            half = 0.5 * gate
            h = ((half * jnp.tanh(half) + half) * up).astype(bf16)
            for c in range(FC):
                hb[g * FC + c] = pltpu.bitcast(_block(h, c), f32)
            return 0
        jax.lax.fori_loop(0, NG, body, 0)

    @pl.when(n == 1)
    def _wait_w2():
        wait(cp_w2)

    @pl.when(jnp.logical_and(n > 0, n < NJOB))
    def _main():
        for i in (Q_, K_, V_):
            project(i, blk == 0)
        for r0 in range(0, RB, AR):
            attend(r0, AR, blk * RB)
        xs[rows(prev), :] += _dot(hidden(0, DS), _cols(w2, 0, NB, slice(0, DS * 128)))

        x1 = out_proj(blk)
        for j in range(NB):
            att[Q_, j, HALO:HALO + RB, :] = _block(x1, j)

        def x1_rows(r0):
            return jnp.concatenate([att[Q_, j, HALO + r0:HALO + r0 + 32, :] for j in range(NB)], axis=1)

        cur = x1_rows(0)
        for r0 in range(0, RB, 32):
            nxt = x1_rows(r0 + 32) if r0 + 32 < RB else None
            ln_store(XF_, r0, cur)
            cur = nxt

        y = xs[rows(prev), :] + _dot(hidden(DS, FB - DS), _cols(w2, 0, NB, slice(DS * 128, F)))
        xs[rows(prev), :] = y
        o_ref[...] = y.astype(bf16)

    @pl.when(n == NJOB)
    def _last():
        def body(c, _):
            ks = pl.ds(pl.multiple_of(c * 896, 128), 896)
            xs[rows(prev), :] += _dot(hidden(c * 7, 7), _cols(w2, 0, NB, ks))
            return 0
        jax.lax.fori_loop(0, F // 896, body, 0)
        o_ref[...] = xs[rows(prev), :].astype(bf16)


@jax.jit
def pallas_interleave_layers__sliding_local_dilated__glu_gated_swiglu__prompt_kernel(
    A_x: jax.Array,
    A_wqkv: jax.Array,
    A_wo: jax.Array,
    B_x: jax.Array,
    B_w1: jax.Array,
    B_w3: jax.Array,
    B_w2: jax.Array,
):
    del B_x
    first_out = (LAYERS - 1) * NBLK + 1
    out = pl.pallas_call(
        _kernel,
        grid=(NJOB + 1,),
        in_specs=[pl.BlockSpec(memory_space=pl.ANY)] * 6,
        out_specs=pl.BlockSpec((RB, D), lambda i: (jnp.maximum(i - first_out, 0), 0)),
        out_shape=jax.ShapeDtypeStruct((S, D), bf16),
        scratch_shapes=[
            *[pltpu.VMEM((NB, D, 128), bf16)] * 4,
            *[pltpu.VMEM((FB, D, 128), bf16)] * 2,
            pltpu.VMEM((NB, F, 128), bf16),
            pltpu.VMEM((S, D), bf16),
            pltpu.VMEM((S + 8, D), f32),
            pltpu.VMEM((7, NB, HALO + RB, 128), f32),
            pltpu.VMEM((FB, RB // 2, 128), f32),
            pltpu.SemaphoreType.DMA((5 + NG + D // QS + 2 * (D // KS),)),
        ],
        compiler_params=pltpu.CompilerParams(
            dimension_semantics=("arbitrary",), vmem_limit_bytes=100 * 1024 * 1024),
    )(A_x.reshape(S, D), A_wqkv, A_wo, B_w1, B_w3, B_w2)
    return out.reshape(1, S, D)
```

```python
import functools

import jax
import jax.numpy as jnp
import jax.experimental.pallas as pl
import jax.experimental.pallas.tpu as pltpu

S, D, F = 2048, 1024, 3584
DH, W, DIL = 32, 8, 2
LAYERS = 2
RB = 256
NBLK = S // RB
NJOB = LAYERS * NBLK
HALO = 16
NB = D // 128
FB = F // 128
NG = 2
FC = FB // NG
DS = 24
AR = 16
QS = 256
KS = D // 2
LOG2E = 1.4426950408889634
Q_, K_, V_, T_, XA_, XF_, O_ = range(7)
f32, bf16 = jnp.float32, jnp.bfloat16


def _ln(x):
    d = x - jnp.mean(x, axis=-1, keepdims=True)
    v = jnp.mean(d * d, axis=-1, keepdims=True)
    return d * jax.lax.rsqrt(v + 1e-5)


def _dot(a, b):
    return jnp.dot(a, b, preferred_element_type=f32)


def _total(terms):
    return functools.reduce(jnp.add, terms)


def _cols(ref, start, count, rows=slice(None)):
    return jnp.concatenate([ref[start + c, rows, :] for c in range(count)], axis=1)


def _block(x, j):
    return x[:, j * 128:(j + 1) * 128]


def _swap_blocks(blocks, axis, unit):
    blocks = list(blocks)
    size = blocks[0].shape[axis]
    pos = jax.lax.broadcasted_iota(jnp.int32, blocks[0].shape, axis)
    for b in range(3):
        dist = unit << b
        low = (pos & dist) == 0
        for c in range(NB):
            if c & (1 << b):
                continue
            lo, hi = blocks[c], blocks[c | (1 << b)]
            blocks[c] = jnp.where(low, lo, pltpu.roll(hi, dist, axis))
            blocks[c | (1 << b)] = jnp.where(low, pltpu.roll(lo, size - dist, axis), hi)
    return blocks


def _kernel(x_hbm, wqkv_hbm, wo_hbm, w1_hbm, w3_hbm, w2_hbm, o_ref,
            wq, wk, wv, wo, w1, w3, w2, xb, xs, att, hb, sems):
    n = pl.program_id(0)
    blk = n % NBLK
    prev = jnp.maximum(n - 1, 0) % NBLK
    wqkv = (wq, wk, wv)
    zero = (n // 4096) * 8

    def rows(b):
        if isinstance(b, int):
            return slice(b * RB, (b + 1) * RB)
        return pl.ds(pl.multiple_of(b * RB, RB), RB)

    def pinned(r0, size):
        return pl.ds(pl.multiple_of(r0 + zero, 8), size)

    def row_copy(lo, hi, sem):
        return [pltpu.make_async_copy(x_hbm.at[pl.ds(lo, hi - lo)], xb.at[pl.ds(lo, hi - lo)], sems.at[sem])]

    def col_copies(src, dst, lo, hi, sem):
        return [pltpu.make_async_copy(src.at[:, pl.ds(c * 128, 128)], dst.at[c], sems.at[sem])
                for c in range(lo, hi)]

    def slab_copies(i, size, sem):
        return [[pltpu.make_async_copy(wqkv_hbm.at[pl.ds(r * size, size), pl.ds(i * D + c * 128, 128)],
                                       wqkv[i].at[c, pl.ds(r * size, size)], sems.at[sem + r])
                 for c in range(NB)] for r in range(D // size)]

    cp_x0, cp_x1, cp_xr = row_copy(0, RB, 0), row_copy(RB, 2 * RB, 1), row_copy(2 * RB, S, 2)
    cp_wo = col_copies(wo_hbm, wo, 0, NB, 3)
    cp_w2 = col_copies(w2_hbm, w2, 0, NB, 4)
    cp_gu = [col_copies(w1_hbm, w1, g * FC, (g + 1) * FC, 5 + g) + col_copies(w3_hbm, w3, g * FC, (g + 1) * FC, 5 + g)
             for g in range(NG)]
    cp_q = slab_copies(Q_, QS, 5 + NG)
    cp_kv = [slab_copies(i, KS, 5 + NG + D // QS + (i - K_) * (D // KS)) for i in (K_, V_)]

    def start(cps):
        for c in cps:
            c.start()

    def wait(cps):
        for c in cps:
            c.wait()

    def wait_one(groups, k):
        for i, cps in enumerate(groups):
            pl.when(k == i)(functools.partial(wait, cps))

    def permute_cols(w, r0, size):
        rs = pl.ds(pl.multiple_of(r0, size), size)
        blocks = _swap_blocks([pltpu.bitcast(w[c, rs, :], jnp.uint32) for c in range(NB)], 1, 2)
        for c in range(NB):
            w[c, rs, :] = pltpu.bitcast(blocks[c], bf16)

    def permute_wo_rows():
        def body(m, _):
            rs = [pl.ds(pl.multiple_of(c * 128 + m * 16, 16), 16) for c in range(NB)]
            blocks = _swap_blocks([pltpu.bitcast(_cols(wo, 0, NB, r), jnp.uint32) for r in rs], 0, 1)
            for r, words in zip(rs, blocks):
                y = pltpu.bitcast(words, bf16)
                for j in range(NB):
                    wo[j, r, :] = _block(y, j)
            return 0
        jax.lax.fori_loop(0, 128 // 16, body, 0)

    def packed(plane):
        return jnp.concatenate([pltpu.bitcast(att[plane, j, 0:RB // 2, :], bf16) for j in range(NB)], axis=1)

    def hidden(c0, count):
        return jnp.concatenate([pltpu.bitcast(hb[c0 + c], bf16) for c in range(count)], axis=1)

    def ln_store(plane, r0, x):
        y = pltpu.bitcast(_ln(x).astype(bf16), f32)
        dst = pinned(r0 // 2, x.shape[0] // 2)
        for j in range(NB):
            att[plane, j, dst, :] = _block(y, j)
        return y

    def ln_first_block(plane):
        def body(i, _):
            r0 = pl.multiple_of(i * 128, 128)
            ln_store(plane, r0, xs[pl.ds(r0, 128), :])
            return 0
        jax.lax.fori_loop(0, RB // 128, body, 0)

    def load_x(lo, hi):
        def body(i, _):
            rs = pl.ds(pl.multiple_of(i * 64, 64), 64)
            xs[rs, :] = xb[rs, :].astype(f32)
            return 0
        jax.lax.fori_loop(lo // 64, hi // 64, body, 0)

    def project(i, first, j0=0, count=NB):
        y = _dot(packed(XA_), _cols(wqkv[i], j0, count))
        for j in range(count):
            yj = _block(y, j)
            if i != Q_:
                halo = jnp.broadcast_to(yj[0:1, :], (HALO, 128))
                if first is not True:
                    halo = jnp.where(first, halo, att[i, j0 + j, RB:RB + HALO, :])
                att[i, j0 + j, 0:HALO, :] = halo
            att[i, j0 + j, HALO:HALO + RB, :] = yj

    def attend(r0, size, pos0):
        static = isinstance(r0, int)
        here = pl.ds(HALO + r0, size)
        q = [att[Q_, j, here, :] for j in range(NB)]
        parts = []
        for w in range(W):
            part = _total(q[j] * att[K_, j, pl.ds(HALO + r0 - DIL * w, size), :] for j in range(NB))
            if w < W - 1:
                att[T_, w, pinned(HALO + r0, 8), :] = part[size - 8:]
            parts.append(part)
        lane = jax.lax.broadcasted_iota(jnp.int32, (size, 128), 1)
        row = jax.lax.broadcasted_iota(jnp.int32, (size, 128), 0)
        even, low = (lane & 1) == 0, (lane & 16) == 0
        logits = []
        for w, a in enumerate(parts):
            a = a + jnp.where(even, pltpu.roll(a, 127, 1), pltpu.roll(a, 1, 1))
            a = a + jnp.where(low, pltpu.roll(a, 112, 1), pltpu.roll(a, 16, 1))
            a = a * (DH ** -0.5 * LOG2E)
            if not static or r0 < DIL * w:
                a = jnp.where(pos0 + r0 + row - DIL * w >= 0, a, -1e9 * LOG2E)
            logits.append(a)
        top = functools.reduce(jnp.maximum, logits)
        e = [jnp.exp2(a - top) for a in logits]
        inv = 1.0 / _total(e)
        for j in range(NB):
            acc = _total(e[w] * att[V_, j, pl.ds(HALO + r0 - DIL * w, size), :] for w in range(W))
            att[O_, j, pinned(r0 // 2, size // 2), :] = pltpu.bitcast((acc * inv).astype(bf16), f32)

    def out_proj(b):
        y = xs[rows(b), :] + _dot(packed(O_), _cols(wo, 0, NB))
        xs[rows(b), :] = y
        return y

    @pl.when(n == 0)
    def _start():
        start(cp_x0 + sum(cp_q, []))
        wait(cp_x0)
        load_x(0, RB)
        ln_first_block(XA_)
        start(sum(cp_kv[0] + cp_kv[1], []))

        def permute_q(r, _):
            wait_one(cp_q, r)
            permute_cols(wq, r * QS, QS)
            return 0
        jax.lax.fori_loop(0, D // QS, permute_q, 0)

        for i in (Q_, K_, V_):
            start((cp_x1 + cp_wo, cp_gu[0], cp_gu[1])[i])

            def half(c, _, i=i):
                if i != V_:
                    wait_one(cp_kv[i], c)
                project(i, True, c * (NB * KS // D), NB * KS // D)
                if i != V_:
                    permute_cols(wqkv[i + 1], c * KS, KS)
                return 0
            jax.lax.fori_loop(0, D // KS, half, 0)

        wait(cp_x1)
        load_x(RB, 2 * RB)
        wait(cp_wo)
        permute_wo_rows()

        def attend_rows(i, _):
            attend(pl.multiple_of(i * 128, 128), 128, 0)
            return 0
        jax.lax.fori_loop(0, RB // 128, attend_rows, 0)
        start(cp_w2 + cp_xr)
        out_proj(0)
        ln_first_block(XF_)

    @pl.when(n == 2)
    def _rest_of_x():
        wait(cp_xr)
        load_x(2 * RB, 3 * RB)

    @pl.when(n > 0)
    def _gate_up():
        fresh = jnp.logical_and(n >= 2, n + 1 < NBLK)
        src, dst = jnp.where(fresh, n + 1, 0), jnp.where(fresh, n + 1, NBLK)

        def body(g, _):
            pl.when(n == 1)(lambda: wait_one(cp_gu, g))
            gate = _dot(packed(XF_), _cols(w1, g * FC, FC))
            for r in range(0, RB // NG, 16):
                r0 = pl.multiple_of(g * (RB // NG) + r, 16)
                y = ln_store(XA_, r0, xs[pl.ds(pl.multiple_of(blk * RB + r0, 16), 16), :])
                xs[pl.ds(pl.multiple_of(dst * RB + r0, 16), 16), :] = (
                    xb[pl.ds(pl.multiple_of(src * RB + r0, 16), 16), :].astype(f32))
                xs[pinned(S + RB, 8), 0:128] = y[0:8, 0:128]
            up = _dot(packed(XF_), _cols(w3, g * FC, FC))
            half = 0.5 * gate
            h = ((half * jnp.tanh(half) + half) * up).astype(bf16)
            for c in range(FC):
                hb[g * FC + c] = pltpu.bitcast(_block(h, c), f32)
            return 0
        jax.lax.fori_loop(0, NG, body, 0)

    @pl.when(n == 1)
    def _wait_w2():
        wait(cp_w2)

    @pl.when(jnp.logical_and(n > 0, n < NJOB))
    def _main():
        for i in (Q_, K_, V_):
            project(i, blk == 0)
        for r0 in range(0, RB, AR):
            attend(r0, AR, blk * RB)
        xs[rows(prev), :] += _dot(hidden(0, DS), _cols(w2, 0, NB, slice(0, DS * 128)))

        x1 = out_proj(blk)
        for j in range(NB):
            att[Q_, j, HALO:HALO + RB, :] = _block(x1, j)

        def x1_rows(r0):
            return jnp.concatenate([att[Q_, j, HALO + r0:HALO + r0 + 32, :] for j in range(NB)], axis=1)

        cur = x1_rows(0)
        for r0 in range(0, RB, 32):
            nxt = x1_rows(r0 + 32) if r0 + 32 < RB else None
            ln_store(XF_, r0, cur)
            cur = nxt

        y = xs[rows(prev), :] + _dot(hidden(DS, FB - DS), _cols(w2, 0, NB, slice(DS * 128, F)))
        xs[rows(prev), :] = y
        o_ref[...] = y.astype(bf16)

    @pl.when(n == NJOB)
    def _last():
        def body(c, _):
            ks = pl.ds(pl.multiple_of(c * 896, 128), 896)
            xs[rows(prev), :] += _dot(hidden(c * 7, 7), _cols(w2, 0, NB, ks))
            return 0
        jax.lax.fori_loop(0, F // 896, body, 0)
        o_ref[...] = xs[rows(prev), :].astype(bf16)


@jax.jit
def pallas_interleave_layers__sliding_local_dilated__glu_gated_swiglu__prompt_kernel(
    A_x: jax.Array,
    A_wqkv: jax.Array,
    A_wo: jax.Array,
    B_x: jax.Array,
    B_w1: jax.Array,
    B_w3: jax.Array,
    B_w2: jax.Array,
):
    del B_x
    first_out = (LAYERS - 1) * NBLK + 1
    out = pl.pallas_call(
        _kernel,
        grid=(NJOB + 1,),
        in_specs=[pl.BlockSpec(memory_space=pl.ANY)] * 6,
        out_specs=pl.BlockSpec((RB, D), lambda i: (jnp.maximum(i - first_out, 0), 0)),
        out_shape=jax.ShapeDtypeStruct((S, D), bf16),
        scratch_shapes=[
            *[pltpu.VMEM((NB, D, 128), bf16)] * 4,
            *[pltpu.VMEM((FB, D, 128), bf16)] * 2,
            pltpu.VMEM((NB, F, 128), bf16),
            pltpu.VMEM((S, D), bf16),
            pltpu.VMEM((S + RB + 8, D), f32),
            pltpu.VMEM((7, NB, HALO + RB, 128), f32),
            pltpu.VMEM((FB, RB // 2, 128), f32),
            pltpu.SemaphoreType.DMA((5 + NG + D // QS + 2 * (D // KS),)),
        ],
        compiler_params=pltpu.CompilerParams(
            dimension_semantics=("arbitrary",), vmem_limit_bytes=100 * 1024 * 1024),
    )(A_x.reshape(S, D), A_wqkv, A_wo, B_w1, B_w3, B_w2)
    return out.reshape(1, S, D)
```
